```python
import os as _os
_os.environ.setdefault("JAX_PLATFORMS", "cpu")
import jax
import jax.numpy as jnp

def _softmax(x, axis=-1):
    return jax.nn.softmax(x, axis=axis)
def _gelu(x):
    return jax.nn.gelu(x, approximate=True)
def _silu(x):
    return jax.nn.silu(x)
def _sigmoid(x):
    return jax.nn.sigmoid(x)
def _layernorm(x, axis=-1, eps=1e-5):
    m = jnp.mean(x, axis=axis, keepdims=True)
    v = jnp.var(x, axis=axis, keepdims=True)
    return (x - m) / jnp.sqrt(v + eps)
def _scatter_add(tgt, idx, src, axis=0):
    return tgt.at[idx].add(src)
def _segment_sum(src, seg, n):
    return jax.ops.segment_sum(src, seg, n)
class _Rng:
    def __init__(self, key):
        self._k = key
    def _next(self):
        self._k, sub = jax.random.split(self._k)
        return sub
    def normal(self, shape):
        return jax.random.normal(self._next(), shape, dtype=jnp.bfloat16)
    def randint(self, lo, hi, shape):
        return jax.random.randint(self._next(), shape, lo, hi, dtype=jnp.int32)
    def uniform(self, shape, lo=0.0, hi=1.0):
        return jax.random.uniform(self._next(), shape, jnp.bfloat16, lo, hi)
    def permutation(self, n):
        return jax.random.permutation(self._next(), n)


kernel_name = 'interleave_layers__linear_attn_block__mha_block__prompt'

def setup_inputs():
    _rng = _Rng(jax.random.key(int.from_bytes(__import__("os").urandom(4), "little")))
    _w = (lambda a: (lambda t: t.astype(jnp.bfloat16) if jnp.issubdtype(t.dtype, jnp.floating) else t)(jnp.asarray(a)))
    def _A_setup():
        B, S, D = 1, 2048, 1024
        return {
            "x": _w((lambda *s: _rng.normal(s) * 0.05)(B, S, D)),
            "wqkv": _w((lambda *s: _rng.normal(s) * 0.1)(D, 3 * D)),
            "wo": _w((lambda *s: _rng.normal(s) * 0.1)(D, D)),
        }
    _A_in = _A_setup()

    def _B_setup():
        B, S, D, H = 1, 2048, 1024, 32
        return {
            "x": _w((lambda *s: _rng.normal(s) * 0.05)(B, S, D)),
            "wqkv": _w((lambda *s: _rng.normal(s) * 0.1)(D, 3 * D)),
            "wo": _w((lambda *s: _rng.normal(s) * 0.05)(D, D)),
        }
    _B_in = _B_setup()

    return {
        "A_x": _A_in["x"],
        "A_wqkv": _A_in["wqkv"],
        "A_wo": _A_in["wo"],
        "B_x": _B_in["x"],
        "B_wqkv": _B_in["wqkv"],
        "B_wo": _B_in["wo"],
    }

def reference(A_x, A_wqkv, A_wo, B_x, B_wqkv, B_wo):
    def _A_ref(x, wqkv, wo):
        B, S, D = x.shape
        H = 32; Dh = D // H
        qkv = (lambda x, *d: x.transpose(*d))((x @ wqkv).reshape(B, S, 3, H, Dh), 2, 0, 3, 1, 4)
        q, k, v = qkv[0], qkv[1], qkv[2]
        phi = lambda t: jnp.where(t > 0, t + 1, jnp.exp(t)) + 1e-6
        pq, pk = phi(q), phi(k)
        kv = jnp.einsum("bhsd,bhse->bhde", pk, v)
        z = jnp.einsum("bhsd->bhd", pk)
        num = jnp.einsum("bhqd,bhde->bhqe", pq, kv)
        den = jnp.einsum("bhqd,bhd->bhq", pq, z)[..., None] + 1e-6
        o = num / den
        return (lambda x, *d: x.transpose(*d))(o, 0, 2, 1, 3).reshape(B, S, D) @ wo

    def _B_ref(x, wqkv, wo):
        B, S, D = x.shape
        H = 32
        Dh = D // H
        qkv = (lambda x, *d: x.transpose(*d))((x @ wqkv).reshape(B, S, 3, H, Dh), 2, 0, 3, 1, 4)
        q, k, v = qkv[0], qkv[1], qkv[2]
        scores = jnp.einsum("bhqd,bhkd->bhqk", q, k) * (Dh ** -0.5)
        p = _softmax(scores, axis=-1)
        o = jnp.einsum("bhqk,bhkd->bhqd", p, v)
        return (lambda x, *d: x.transpose(*d))(o, 0, 2, 1, 3).reshape(B, S, D) @ wo

    x = A_x
    x = x + _A_ref(_layernorm(x, axis=-1), A_wqkv, A_wo)
    x = x + _B_ref(_layernorm(x, axis=-1), B_wqkv, B_wo)
    x = x + _A_ref(_layernorm(x, axis=-1), A_wqkv, A_wo)
    x = x + _B_ref(_layernorm(x, axis=-1), B_wqkv, B_wo)
    return x
```

```python
import math

import jax
import jax.numpy as jnp
import numpy as np
from jax import lax
import jax.experimental.pallas as pl
import jax.experimental.pallas.tpu as pltpu

S, D, H, DH = 2048, 1024, 32, 32
G = D // 128
PW = 512
U32, BF, F32 = jnp.uint32, jnp.bfloat16, jnp.float32
NT = (((1,), (1,)), ((), ()))

CFG = dict(TM=256, ACC=1, BQ=512, CK=128, RG=32, DG=1, LAG=1, PH="12345", SPAN=90, TK=2, WIN=20, WIN2=10, FLAG="",
           LAZYW=1, LAZYX=0, AU=2, OFF=2, LEAD=2, NS=4, DL=0, XW=1)


def _quads(x):
    h = len(x) // 2
    return [[r[j * h:(j + 1) * h] for r in x[i * h:(i + 1) * h]] for i in (0, 1) for j in (0, 1)]


def _add(u, v):
    return [[p + q for p, q in zip(ru, rv)] for ru, rv in zip(u, v)]


def _sub(u, v):
    return [[p - q for p, q in zip(ru, rv)] for ru, rv in zip(u, v)]


class Classic:
    lhs_scale = rhs_scale = out_scale = ((1.0, 1.0), (1.0, 1.0))
    rhs_factor = (1.0,) * 7

    @staticmethod
    def lhs(a11, a12, a21, a22):
        return (_sub(a21, a11), _add(a21, a22), a22, _sub(a12, a22), _add(a11, a22), _add(a11, a12), a11)

    @staticmethod
    def rhs(b11, b12, b21, b22):
        return (_add(b11, b12), b11, _sub(b21, b11), _add(b21, b22), _add(b11, b22), b22, _sub(b12, b22))

    @staticmethod
    def step(m, v, a, emit):
        if m == 0:
            a["11"] = v
        elif m == 1:
            a["11"] = a["11"] - v
            a["10"] = v
        elif m == 2:
            emit(1, 0, a["10"] + v)
            a["00"] = v
        elif m == 3:
            a["00"] = a["00"] + v
        elif m == 4:
            a["00"] = a["00"] + v
            a["11"] = a["11"] + v
        elif m == 5:
            emit(0, 0, a["00"] - v)
            a["01"] = v
        else:
            emit(0, 1, a["01"] + v)
            emit(1, 1, a["11"] + v)


class Balanced:
    lhs_scale = rhs_scale = ((1.0, 0.5), (2.0, 1.0))
    out_scale = ((1.0, 2.0), (0.5, 1.0))
    rhs_factor = (0.5, 0.5, 1.0, 0.5, 0.5, 0.5, 0.5)

    @staticmethod
    def _g(z11, u, v, z22):
        t, w = _add(z11, z22), _add(u, v)
        return dict(t=t, g12=_sub(z11, u), g13=_add(z11, u), g23=_sub(z22, u), g32=_add(z22, u),
                    g21=_sub(t, w), g31=_add(t, w))

    @classmethod
    def lhs(cls, *q):
        g = cls._g(*q)
        return [g[k] for k in ("g13", "g12", "t", "g23", "g32", "g31", "g21")]

    @classmethod
    def rhs(cls, *q):
        g = cls._g(*q)
        return [g[k] for k in ("g32", "g23", "t", "g31", "g21", "g12", "g13")]

    @staticmethod
    def step(m, v, a, emit):
        if m == 0:
            a["p"] = v
        elif m == 1:
            a["s"] = a["p"] + v
            a["d"] = a["p"] - v
            emit(0, 1, a["d"])
        elif m == 2:
            a["t"] = v - a["s"]
        elif m == 3:
            a["c"] = a["t"] - v
            a["d"] = a["d"] + v
        elif m == 4:
            emit(0, 0, a["c"] - v)
            a["d"] = a["d"] - v
        elif m == 5:
            a["c"] = a["t"] - v
            a["d"] = a["d"] + v
        else:
            emit(1, 1, a["c"] - v)
            emit(1, 0, a["d"] - v)


def _scale(tab, i, j):
    return tab[i & 1][j & 1] * tab[i >> 1][j >> 1]


def _mul(v, s):
    return v if s == 1.0 else v * s


def _same(v):
    return v


def _now(pre=0):
    return None


def _gmul(v, s, tok):
    if tok is None:
        return _mul(v, s)
    sv = pltpu.bitcast(tok | np.float32(s).view(np.uint32), F32)
    return v * jnp.tile(sv, (v.shape[0] // 8, 1))


def _seven(f, tiles, m, tok=None):
    top = f(*_quads([[tiles[i, j] for j in range(4)] for i in range(4)]))[m]
    top[0][0] = _gmul(top[0][0], 1.0, tok)
    return [v[0][0] for v in f(*_quads(top))]


def _combine(alg, prod, emit):
    outer = {}
    for m in range(7):
        def inner(i, j, v, m=m):
            alg.step(m, v, outer.setdefault((i, j), {}), lambda ci, cj, r: emit(2 * ci + i, 2 * cj + j, r))
        acc = {}
        for n in range(7):
            alg.step(n, prod(7 * m + n), acc, inner)


def _phi(t):
    return jnp.where(t > 0, t + 1.0, jnp.exp(t)) + 1e-6


def _pack(v):
    return pltpu.bitcast(v.astype(BF), U32)


def _bf(v):
    return pltpu.bitcast(v, BF)


def build(cfg):
    TM = cfg["TM"]
    BQ, CK, RG, DG, LAG = cfg["BQ"], cfg["CK"], cfg["RG"], cfg["DG"], cfg["LAG"]
    NB, NQ, NC = S // TM, S // BQ, S // CK
    NP = 49
    MB, KB = TM // 4, D // 4
    QSCALE = DH ** -0.5 * math.log2(math.e)
    ALG_A = Balanced if cfg["ACC"] else Classic
    PH = str(cfg["PH"])

    def kernel(x_hbm, aqkv_hbm, awo_hbm, bqkv_hbm, bwo_hbm, out_hbm,
               xs, raw, wa, wb, xa, xb, fa, fb, q_s, k_s, vt_s, o_s, kv_s, z_s, kz_s, m_s, ot_s,
               sem_x, sem_w, *sbuf):
        X, F = (xa, xb), (fa, fb)

        def at(start, n):
            return pl.ds(start if isinstance(start, int) else pl.multiple_of(start, n), n)

        def x_copy(i):
            return pltpu.make_async_copy(x_hbm.at[at(i * TM, TM)], xs.at[at(i * TM, TM)], sem_x.at[i])

        def out_copy(i):
            return pltpu.make_async_copy(xs.at[at(i * TM, TM)], out_hbm.at[at(i * TM, TM)], sem_x.at[i])

        def w_copy(p):
            src, c = ((aqkv_hbm, p), (awo_hbm, p - 6), (bqkv_hbm, p - 8), (bwo_hbm, p - 14))[
                (p >= 6) + (p >= 8) + (p >= 14)]
            return pltpu.make_async_copy(src.at[:, pl.ds(c * PW, PW)], raw.at[p], sem_w.at[p])

        def prep_rows(alg, p, r16, dst, pd, z=0):
            tiles = {}
            def task(m, late):
                if cfg["LAZYW"] or not tiles:
                    for ki in range(4):
                        for n2 in range(2):
                            w = raw[p + z * (m + 1), at(r16 * 16 + ki * KB, 16), pl.ds(n2 * 256, 256)].astype(F32)
                            for nj in (2 * n2, 2 * n2 + 1):
                                tiles[ki, nj] = _mul(w[:, nj % 2 * 128:(nj % 2 + 1) * 128],
                                                     _scale(alg.rhs_scale, ki, nj) * alg.rhs_factor[0] ** 2)
                for n, v in enumerate(_seven(alg.rhs, tiles, m, late())):
                    f = alg.rhs_factor[m] * alg.rhs_factor[n] / alg.rhs_factor[0] ** 2
                    dst[pd, 7 * m + n, at(r16 * 8, 8), :] = _pack(_mul(v, f))
                return lambda: dst[pd + z, 7 * m + 6, at(r16 * 8, 8), :]
            return [lambda late=_now, m=m: task(m, late) for m in range(7)]

        def prep_loop(p):
            def body(i, c):
                for t in prep_rows(ALG_A, p, i, wa, p):
                    t()
                return c
            lax.fori_loop(0, KB // 16, body, 0)

        def put_ops(alg, src, row0, dst, z):
            def piece(r, c):
                tiles = {}
                def task(m, late):
                    if cfg["LAZYX"] or not tiles:
                        for mi in range(4):
                            for kj in range(4):
                                tiles[mi, kj] = src[2 * kj + c + z * (m + 1), at(row0 + mi * MB + r, 16), :]
                    for n, v in enumerate(_seven(alg.lhs, tiles, m, late())):
                        dst[0, 7 * m + n, pl.ds(r // 2, 8), pl.ds(c * 128, 128)] = _pack(v)
                    return lambda: dst[z, 7 * m + 6, pl.ds(r // 2, 8), pl.ds(c * 128, 128)]
                return [lambda late=_now, m=m: task(m, late) for m in range(7)]
            return [t for r in range(0, MB, 16) for c in range(2) for t in piece(r, c)]

        class Pacer:
            def __init__(self, z, shared, nproj, lists, win):
                self.z, self.lists, self.win = z, lists, win
                self.hist, self.due = shared
                self.n = nproj * 2 * NP * cfg["SPAN"] // 100
                self.t, self.done, self.probes = 0, [0] * len(lists), {}
                self.zero = jnp.full((8, 128), z, jnp.int32).astype(U32)

            def late(self):
                if len(self.hist) < self.win:
                    return None
                return pltpu.bitcast(self.hist[-self.win][:8], U32) & self.zero

            def deadline(self, v):
                if cfg["DL"]:
                    self.due.append((len(self.hist) + cfg["DL"], v))

            def tick(self, lhs):
                if self.t % cfg["TK"] == 0:
                    toks = [probe() for probe in self.probes.values()]
                    self.probes = {}
                    while self.due and self.due[0][0] <= len(self.hist):
                        toks.append(self.due.pop(0)[1]())
                    if toks:
                        tok = self.zero
                        for v in toks:
                            tok = tok & v
                        head = jnp.concatenate([lhs[:8, :128] | tok, lhs[:8, 128:]], axis=1)
                        lhs = jnp.concatenate([head, lhs[8:]], axis=0)
                self.t += 1
                for k, tasks in enumerate(self.lists):
                    while self.done[k] < min(len(tasks), self.t * len(tasks) // self.n):
                        probe = tasks[self.done[k]](self.late)
                        if isinstance(probe, tuple):
                            self.deadline(probe[0])
                        elif probe is not None:
                            self.probes[k] = probe
                        self.done[k] += 1
                return lhs

        def proj(src, p0, emit, pace, mult=1.0):
            alg = ALG_A if p0 < 6 else Classic
            for p in (p0, p0 + 1):
                z = pace.z * (p + 1)
                def prod(t):
                    w = wa[p + z, t] if p < 6 else wb[p - 6 + z, t]
                    r = jnp.dot(_bf(pace.tick(src[z, t])), _bf(w), preferred_element_type=F32)
                    pace.hist.append(r)
                    return r
                _combine(alg, prod, lambda mi, nj, v: emit(
                    mi, 4 * (p - p0) + nj, _mul(v, mult * _scale(alg.out_scale, mi, nj))))

        def ln_block(alg, i, dst, z):
            def task(r, late):
                x = xs[at(i * TM + r, 8), :].astype(F32)
                x = jnp.concatenate([_gmul(x[:, :128], 1.0, late()), x[:, 128:]], axis=1)
                xc = x - jnp.mean(x, axis=-1, keepdims=True)
                rs = lax.rsqrt(jnp.mean(xc * xc, axis=-1, keepdims=True) + 1e-5)
                for g in range(G):
                    dst[g, pl.ds(r, 8), :] = xc[:, g * 128:(g + 1) * 128] * _mul(
                        rs, _scale(alg.lhs_scale, r // MB, g // 2))
                return lambda: pltpu.bitcast(dst[G - 1 + z, pl.ds(r, 8), :], U32)
            return [lambda late=_now, r=r: task(r, late) for r in range(0, TM, 8)]

        def natural(dst, i, f):
            def emit(mi, g, v):
                dst[g, at((i * TM + mi * MB) // 2, MB // 2), :] = _pack(f(g, v))
            return emit

        def transposed(dst, i, pace, f=_same):
            hold = {}
            def emit(mi, g, v):
                hold[mi, g] = f(v)
                if (mi ^ 1, g) in hold:
                    vv = jnp.concatenate([hold.pop((mi & 2, g)), hold.pop((mi | 1, g))], axis=0)
                    c = pl.ds((mi & 2) * MB, 2 * MB)
                    dst[g, i, :, c] = _pack(vv.T)
                    pace.deadline(lambda: dst[g + pace.z, i, :8, c])
            return emit

        def residual(i):
            def emit(mi, g, v):
                r, c = at(i * TM + mi * MB, MB), pl.ds(g * 128, 128)
                xs[r, c] = (xs[r, c].astype(F32) + v).astype(BF)
            return emit

        def lin_kv(i, src, pace):
            zs = {}
            def fk(g, v):
                pk = _phi(v)
                part = jnp.sum(pk.reshape(MB // 8, 8, 128), axis=0)
                zs[g] = part if g not in zs else zs[g] + part
                return pk
            proj(src, 4, transposed(vt_s, i, pace), pace)
            proj(src, 2, natural(k_s, i, fk), pace)
            for g in range(G):
                z_s[g] += zs[g]

        def lin_acc(i, z):
            def task(g):
                kv_s[g] += jnp.dot(_bf(vt_s[g + z, i]), _bf(k_s[g + z, at(i * (TM // 2), TM // 2), :]),
                                   preferred_element_type=F32)
            return [lambda gate=_same, g=g: task(g) for g in range(G)]

        def lin_q(i, src, pace):
            proj(src, 0, transposed(q_s, i, pace, _phi), pace)

        def lin_mid():
            def task(g):
                row = lax.broadcasted_iota(jnp.int32, (128, 128), 0)
                col = lax.broadcasted_iota(jnp.int32, (128, 128), 1) // DH
                kz_s[g, :64, :] = _pack(jnp.where(row // DH == col, kv_s[g], 0.0))
                zsum = jnp.broadcast_to(jnp.sum(z_s[g], axis=0, keepdims=True), (16, 128))
                kz_s[g, 64:, :] = _pack(jnp.where(row[:16] == col[:16], zsum, 0.0))
            return [lambda gate=_same, g=g: task(g) for g in range(G)]

        def lin_o(i, dst, z):
            def task(g):
                nd = jnp.dot(_bf(kz_s[g + z]), _bf(q_s[g + z, i]), preferred_element_type=F32)
                inv = 1.0 / (nd[128:136] + 1e-6)
                ot = jnp.concatenate([nd[h * DH:(h + 1) * DH] * inv[h:h + 1] for h in range(4)], axis=0)
                dst[g] = ot.T
                return (lambda: pltpu.bitcast(dst[g + z, :8], U32),)
            return [lambda gate=_same, g=g: task(g) for g in range(G)]

        def lin_phase(rep, prep):
            def block(i, u, z, hist, nxt, last=False):
                lists = []
                if cfg["XW"]:
                    lists.append([t for r in range(KB // 16) for t in prep_rows(Classic, 6 + i, r, wb, i, z)])
                if not last:
                    lists.append(put_ops(ALG_A, F[1 - u], 0, X[1 - u], z))
                if nxt:
                    lists.append(ln_block(ALG_A, i + 2, F[u], z))
                pace = Pacer(z, hist, 2 if last else 3, lists, cfg["WIN"])
                lin_kv(i, X[u], pace)
                if last:
                    idle = [lambda gate: None]
                    pace = Pacer(z, hist, 1, [lin_acc(i, z) + lin_mid() + lin_o(0, fa, z) + lin_o(1, fb, 2 * z) + idle * 4
                                              + put_ops(Classic, fa, 0, xa, z)], cfg["WIN2"])
                lin_q(i, X[u], pace)
                if not last:
                    for t in lin_acc(i, z):
                        t()
            def body(it, c):
                for k in range(NB // 2 - 1):
                    @pl.when((rep == 0) & (it == k))
                    def _():
                        for cp in (x_copy(2 * k + 2), x_copy(2 * k + 3), w_copy(6 + 2 * k), w_copy(7 + 2 * k)):
                            cp.wait()
                        if k == 0:
                            for cp in [x_copy(i) for i in range(4, NB)] + [w_copy(p) for p in range(8, 16)]:
                                cp.start()
                        if k == NB // 2 - 2:
                            for p in range(12, 16):
                                w_copy(p).wait()
                hist = ([], [])
                for u in range(2):
                    block(2 * it + u, u, it // (NB + u), hist, True)
                return c
            with sc("P1loop"):
                lax.fori_loop(0, NB // 2 - 1, body, 0)
            hist = ([], [])
            block(NB - 2, 0, rep // 2, hist, False)
            block(NB - 1, 1, rep // 3, hist, False, True)

        def out_phase(rep, p0, stage, store, alg_next):
            hist = ([], [])
            for i in range(NB):
                u, z = i % 2, rep // (2 + i)
                if i == NB - 1 or stage is not None:
                    lists = [put_ops(alg_next if i == NB - 1 else Classic, F[1 - u], 0, X[1 - u], z)]
                else:
                    lists = [put_ops(Classic, o_s, (i + 1) * TM, X[1 - u], z)]
                if i >= NB - 2:
                    lists.append(ln_block(alg_next, i + 2 - NB, F[u], z))
                elif stage is not None:
                    lists.append(stage(i + 2, F[u], z))
                proj(X[u], p0, residual(i), Pacer(z, hist, 1, lists, cfg["WIN"] if i >= NB - 2 else cfg["WIN2"]))
                if store:
                    out_copy(i).start()

        def mha_phase():
            def body(it, c):
                hist = ([], [])
                for u in range(2):
                    i, z = 2 * it + u, it // (NB + u)
                    pace = Pacer(z, hist, 3, [put_ops(Classic, F[1 - u], 0, X[1 - u], z),
                                              ln_block(Classic, jnp.minimum(i + 2, NB - 1), F[u], z)], cfg["WIN"])
                    proj(X[u], 12, transposed(vt_s, i, pace), pace)
                    proj(X[u], 8, transposed(q_s, i, pace), pace, QSCALE)
                    proj(X[u], 10, natural(k_s, i, lambda g, v: v), pace)
                return c
            lax.fori_loop(0, NB // 2, body, 0)

        def attn_stream(qk, c0, c1, pv, m, mx, z, tasks=()):
            gpc, ns = CK // RG, cfg["NS"]
            ms, outs, sres, ps = [m], [], {}, {}
            st = dict(mx=mx, gate=None, acc=None, l=None, drained=c0 * gpc)

            def score_ref(hh, row):
                return sbuf[hh % 2 * ns + row // (S // ns)], row % (S // ns)

            def qk_mm(ci):
                t, c = divmod(ci, NC)
                g, j, hh = qk[t]
                kc = _bf(k_s[g + z * (t + 1), pl.ds(c * CK // 2, CK // 2), :])
                q = jnp.concatenate([q_s[g + z * (c + 1), j * (BQ // TM) + b, pl.ds(hh * DH // 2, DH // 2), :]
                                     for b in range(BQ // TM)], axis=1)
                q = jnp.concatenate([q if h == hh else jnp.zeros_like(q) for h in range(4)], axis=0)
                sres[ci] = jnp.dot(kc, _bf(q), preferred_element_type=F32)

            def drain(upto):
                while st["drained"] < min(upto, c1 * gpc):
                    gi = st["drained"]
                    st["drained"] += 1
                    t, r = divmod(gi, NC * gpc)
                    for r8 in range(0, RG, 8):
                        o = gi % gpc * RG + r8
                        sr = sres[gi // gpc][o:o + 8]
                        ref, row = score_ref(qk[t][2], r * RG + r8)
                        ref[0, pl.ds(row, 8), :] = sr
                        st["mx"] = sr if st["mx"] is None else jnp.maximum(st["mx"], sr)
                    st["gate"] = st["mx"]
                    if r == NC * gpc - 1:
                        ms.append(jnp.broadcast_to(jnp.max(st["mx"], axis=0, keepdims=True), (8, BQ)))
                        st["mx"] = None

            def exps(ci):
                t, c = divmod(ci, NC)
                parts = {}
                for k in reversed(range(gpc)):
                    drain((ci + c0) * gpc - k - cfg["LEAD"])
                    mm = ms[t]
                    if st["gate"] is not None:
                        mm = jnp.minimum(mm, jnp.maximum(mm, st["gate"]))
                    ref, row = score_ref(pv[t][1], c * CK + k * RG)
                    p = jnp.exp2(ref[z * (t + 1), pl.ds(row, RG), :].reshape(RG // 8, 8, BQ) - mm[None])
                    lc = jnp.sum(p, axis=0)
                    st["l"] = lc if st["l"] is None else st["l"] + lc
                    parts[k] = p.reshape(RG, BQ)
                ps[ci] = jnp.concatenate([parts[k] for k in range(gpc)], axis=0).astype(BF)

            def pv_mm(ci):
                t, c = divmod(ci, NC)
                g, hh = pv[t]
                vc = vt_s[g, c * CK // TM, pl.ds(hh * DH // 2, DH // 2), pl.ds(c * CK % TM, CK)]
                o = jnp.dot(_bf(vc), ps.pop(ci), preferred_element_type=F32)
                st["acc"] = o if st["acc"] is None else st["acc"] + o
                if c == NC - 1:
                    outs.append(st["acc"] * (1.0 / jnp.sum(st["l"], axis=0, keepdims=True)))
                    st["acc"] = st["l"] = None

            def gate():
                return pltpu.bitcast(st["gate"][:, :128], U32) & jnp.full((8, 128), z, jnp.int32).astype(U32)

            for n in range(max(c1 - c0, len(pv) * NC)):
                if n >= 4 and tasks:
                    span = (c1 - c0) * 7 // 8 - 4
                    for t in tasks[(n - 4) * len(tasks) // span:(n - 3) * len(tasks) // span]:
                        t(gate)
                if c0 + n < c1:
                    qk_mm(c0 + n)
                if n < len(pv) * NC:
                    exps(n)
                    pv_mm(n)
            drain(c1 * gpc)
            return ms[-1], st["mx"], outs

        def put_o(i, u):
            o_s[i >> 2, at((i & 3) * BQ, BQ), :] = ot_s[u].T

        def attention(rep):
            n, au, off = G * NQ, cfg["AU"], cfg["OFF"]
            m_s[0], m_s[1], _ = attn_stream([(0, 0, 0), (0, 0, 1)], 0, NC + off, [], None, None, rep // 2)
            ot_s[...] = jnp.zeros_like(ot_s)

            def body(it, z, last):
                qk, pv, tasks = [], [], []
                for u in range(au):
                    i = it * au + u
                    put_o(jnp.maximum(i - au, 0), u)
                    tasks += prep_rows(Classic, 14 + (i >> 4), i & 15, wb, 8 + (i >> 4), z)
                    pv += [(i >> 2, hh) for hh in range(4)]
                    qk += [(i >> 2, i & 3, hh) for hh in range(4)]
                if last:
                    tasks += put_ops(Classic, o_s, 0, xa, z)
                i = (it + 1) * au
                qk = qk[1:] + [(i >> 2, i & 3, 0), (i >> 2, i & 3, 1)]
                m, mx, outs = attn_stream(qk, off, (len(pv) - 1) * NC if last else len(pv) * NC + off, pv,
                                          m_s[0], m_s[1], z, tasks)
                if not last:
                    m_s[0], m_s[1] = m, mx
                for t, o in enumerate(outs):
                    ot_s[t // 4, pl.ds(t % 4 * DH, DH), :] = o
                return z
            with sc("P4loop"):
                lax.fori_loop(0, n // au - 1, lambda i, z: body(i, z, False), rep // 2)
            if len(PH) < 5:
                return
            body(n // au - 1, rep // 2, True)
            for u in range(au):
                put_o(n - au + u, u)

        x_copy(0).start()
        x_copy(1).start()
        first = [w_copy(p) for p in (4, 5, 2, 3, 0, 1)] + [x_copy(2), x_copy(3), w_copy(6), w_copy(7)]
        first[0].start()
        x_copy(0).wait()
        first[1].start()
        x_copy(1).wait()
        first[2].start()
        for t in ln_block(ALG_A, 0, fa, 0) + ln_block(ALG_A, 1, fb, 0) + put_ops(ALG_A, fa, 0, xa, 0):
            t()
        for n, p in enumerate((4, 5, 2, 3, 0, 1)):
            first[n].wait()
            for cp in first[n + 3:n + 4] if n < 3 else first[2 * n:2 * n + 2]:
                cp.start()
            prep_loop(p)

        import contextlib
        sc = (lambda n: jax.named_scope(n)) if cfg.get("PROF") else (lambda n: contextlib.nullcontext())

        def layer_pair(rep, c):
            if "1" in PH:
                kv_s[...] = jnp.zeros_like(kv_s)
                z_s[...] = jnp.zeros_like(z_s)
                with sc("P1"):
                    lin_phase(rep, True)

            @pl.when(rep == 1)
            def _():
                for i in range(NB):
                    out_copy(i).wait()
            if "2" in PH:
                with sc("P2"):
                    out_phase(rep, 6, lin_o, False, Classic)
            if "3" in PH:
                with sc("P3"):
                    mha_phase()
            if "4" in PH:
                with sc("P4"):
                    attention(rep)
            if "5" in PH:
                with sc("P5"):
                    out_phase(rep, 14, None, True, ALG_A)
            if len(PH) < 5:
                u = q_s[rep, rep, :8, :128] | k_s[rep, :8] | vt_s[rep, rep, :8, :128] | wb[rep, rep, :8] | xa[0, rep, :8, :128].astype(F32).astype(jnp.int32).astype(U32)
                f = pltpu.bitcast(u, F32) + kv_s[rep, :8] + z_s[rep] + o_s[rep, :8] + fa[rep, :8] + fb[rep, :8]
                xs[:8, :128] = f.astype(BF)
            return c
        lax.fori_loop(0, 2, layer_pair, 0)
        for i in range(NB):
            out_copy(i).wait()

    any_spec = pl.BlockSpec(memory_space=pl.ANY)
    return pl.pallas_call(
        kernel,
        out_shape=jax.ShapeDtypeStruct((S, D), BF),
        in_specs=[any_spec] * 5,
        out_specs=any_spec,
        scratch_shapes=[
            pltpu.VMEM((S, D), BF),
            pltpu.VMEM((16, D, PW), BF),
            pltpu.VMEM((6, NP, KB // 2, 128), U32),
            pltpu.VMEM((10, NP, KB // 2, 128), U32),
            pltpu.VMEM((1, NP, MB // 2, KB), U32),
            pltpu.VMEM((1, NP, MB // 2, KB), U32),
            pltpu.VMEM((G, TM, 128), F32),
            pltpu.VMEM((G, TM, 128), F32),
            pltpu.VMEM((G, NB, 64, TM), U32),
            pltpu.VMEM((G, S // 2, 128), U32),
            pltpu.VMEM((G, NB, 64, TM), U32),
            pltpu.VMEM((G, S, 128), F32),
            pltpu.VMEM((G, 128, 128), F32),
            pltpu.VMEM((G, 8, 128), F32),
            pltpu.VMEM((G, 72, 128), U32),
            pltpu.VMEM((2, 8, BQ), F32),
            pltpu.VMEM((cfg["AU"], 128, BQ), F32),
            pltpu.SemaphoreType.DMA((NB,)),
            pltpu.SemaphoreType.DMA((16,)),
        ] + [pltpu.VMEM((1, S // cfg["NS"], BQ), F32)] * (2 * cfg["NS"]),
        compiler_params=pltpu.CompilerParams(vmem_limit_bytes=120 * 2 ** 20,
                                             flags={cfg["FLAG"]: True} if cfg["FLAG"] else None),
    )


@jax.jit
def pallas_interleave_layers__linear_attn_block__mha_block__prompt_kernel(
    A_x: jax.Array,
    A_wqkv: jax.Array,
    A_wo: jax.Array,
    B_x: jax.Array,
    B_wqkv: jax.Array,
    B_wo: jax.Array,
):
    del B_x
    out = build(CFG)(A_x.reshape(S, D), A_wqkv, A_wo, B_wqkv, B_wo)
    return out.reshape(A_x.shape)
```

```python
import math

import jax
import jax.numpy as jnp
from jax import lax
import jax.experimental.pallas as pl
import jax.experimental.pallas.tpu as pltpu

S, D, DH = 2048, 1024, 32
G = D // 128
TM = 256
NB = S // TM
MB = TM // 4
NP = 49
PW = 512
BQ, CK, RG = 512, 128, 16
NQ, NC = S // BQ, S // CK
NS = 4
QSCALE = DH ** -0.5 * math.log2(math.e)
U32, BF, F32 = jnp.uint32, jnp.bfloat16, jnp.float32

CFG = dict(PH="12345", TK=2, DY=6, WIN1=8, WIN2=6, WIN3=12, LW=9, LEAD=0, MP=3, L1=66, A0=70, A1=98, W1=96, O1=94,
           S1=99, WIN0=2, DY0=5, H0=50, NV=4, KD=1, E1=100, HG=4, C0=45, C1=94, C2=98, SP=1)


class Classic:
    lhs_scale = rhs_scale = out_scale = ((1.0, 1.0), (1.0, 1.0))
    lhs = (lambda q: q(1, 0) - q(0, 0), lambda q: q(1, 0) + q(1, 1), lambda q: q(1, 1),
           lambda q: q(0, 1) - q(1, 1), lambda q: q(0, 0) + q(1, 1), lambda q: q(0, 0) + q(0, 1),
           lambda q: q(0, 0))
    rhs = (lambda q: q(0, 0) + q(0, 1), lambda q: q(0, 0), lambda q: q(1, 0) - q(0, 0),
           lambda q: q(1, 0) + q(1, 1), lambda q: q(0, 0) + q(1, 1), lambda q: q(1, 1),
           lambda q: q(0, 1) - q(1, 1))

    @staticmethod
    def step(m, v, a, emit):
        if m == 0:
            a["d"] = v
        elif m == 1:
            a["d"] = a["d"] - v
            a["c"] = v
        elif m == 2:
            emit(1, 0, a["c"] + v)
            a["c"] = v
        elif m == 3:
            a["c"] = a["c"] + v
        elif m == 4:
            a["c"] = a["c"] + v
            a["d"] = a["d"] + v
        elif m == 5:
            emit(0, 0, a["c"] - v)
            a["c"] = v
        else:
            emit(0, 1, a["c"] + v)
            emit(1, 1, a["d"] + v)


def _diag(q):
    return q(0, 0) + q(1, 1)


class Balanced:
    lhs_scale = ((0.5, 0.25), (1.0, 0.5))
    rhs_scale = ((1.0, 0.5), (2.0, 1.0))
    out_scale = ((1.0, 2.0), (0.5, 1.0))
    lhs = (lambda q: q(0, 0) + q(0, 1), lambda q: q(0, 0) - q(0, 1), _diag,
           lambda q: q(1, 1) - q(0, 1), lambda q: q(1, 1) + q(0, 1),
           lambda q: _diag(q) + (q(0, 1) + q(1, 0)), lambda q: _diag(q) - (q(0, 1) + q(1, 0)))
    rhs = (lhs[4], lhs[3], lambda q: 2.0 * _diag(q), lhs[5], lhs[6], lhs[1], lhs[0])

    @staticmethod
    def step(m, v, a, emit):
        if m == 0:
            a["p"] = v
        elif m == 1:
            a["s"] = a["p"] + v
            a["d"] = a["p"] - v
            emit(0, 1, a["d"])
        elif m == 2:
            a["t"] = v - a["s"]
        elif m in (3, 5):
            a["c"] = a["t"] - v
            a["d"] = a["d"] + v
        elif m == 4:
            emit(0, 0, a["c"] - v)
            a["d"] = a["d"] - v
        else:
            emit(1, 1, a["c"] - v)
            emit(1, 0, a["d"] - v)


def _scale(table, i, j):
    return table[i >> 1][j >> 1] * table[i & 1][j & 1]


def _mul(v, s):
    return v if s == 1.0 else v * s


def _memo(f):
    seen = {}
    def g(*key):
        if key not in seen:
            seen[key] = f(*key)
        return seen[key]
    return g


def _now():
    return None


def _after(v, token):
    return v if token is None else pltpu.bitcast(pltpu.bitcast(v, U32) | token, F32)


def _leaves(forms, quad, m, token):
    top = forms[m](quad)
    def tile(i, j):
        r, c = 16 * i, slice(128 * j, 128 * j + 128)
        if i != j or token is None:
            return top[r:r + 16, c]
        return jnp.concatenate([_after(top[r:r + 8, c], token), top[r + 8:r + 16, c]])
    tile = _memo(tile)
    return _pack(jnp.concatenate([f(tile) for f in forms], axis=1))


def _combine(alg, product, emit):
    outer = {}
    for m in range(7):
        def inner(i, j, v, m=m):
            alg.step(m, v, outer.setdefault((i, j), {}), lambda a, b, r: emit(2 * a + i, 2 * b + j, r))
        acc = {}
        for n in range(7):
            alg.step(n, product(m, n), acc, inner)


def _phi(t):
    return jnp.where(t > 0, t + 1.0, jnp.exp(t)) + 1e-6


def _centered(x):
    xc = x - jnp.mean(x, axis=-1, keepdims=True)
    return xc, lax.rsqrt(jnp.mean(xc * xc, axis=-1, keepdims=True) + 1e-5)


def _pack(v):
    return pltpu.bitcast(v.astype(BF), U32)


def _bf(v):
    return pltpu.bitcast(v, BF)


def _at(start, n):
    return pl.ds(start if isinstance(start, int) else pl.multiple_of(start, n), n)


def _zero_tile(z):
    return jnp.full((8, 128), z, jnp.int32).astype(U32)


def _part(tasks, i, n):
    return tasks[i * len(tasks) // n:(i + 1) * len(tasks) // n]


def build(cfg):
    PH = str(cfg["PH"])
    VPU = {4: (1, 5, 9, 13), 5: (1, 4, 7, 10, 13), 6: (1, 4, 7, 9, 12, 14)}[cfg["NV"]]

    class Pacer:
        def __init__(self, z, done, n, lists, window, delay=cfg["DY"]):
            self.z, self.zero, self.done, self.window, self.delay = z, _zero_tile(z), done, window, delay
            self.lists = [(t, max(n * a // 100, 0 if done else 1), n * b // 100) for t, a, b in lists]
            self.t, self.issued, self.probes, self.due = 0, [0] * len(lists), {}, {}
            self.token = _memo(lambda i: pltpu.bitcast(done[i][:8], U32) & self.zero)

        def late(self):
            return self.token(max(0, len(self.done) - self.window)) if self.done else None

        def dot(self, lhs, rhs):
            if self.probes and self.t % cfg["TK"] == 0:
                token = self.zero
                for probe in self.probes.values():
                    token = token & probe()
                self.probes = {}
                self.due[self.t + self.delay] = token
            if self.t in self.due:
                lhs = jnp.concatenate([lhs[:8] | jnp.tile(self.due.pop(self.t), (1, 2)), lhs[8:]])
            self.t += 1
            for k, (tasks, a, b) in enumerate(self.lists):
                while self.issued[k] < min(len(tasks), (self.t - a) * len(tasks) // (b - a)):
                    probe = tasks[self.issued[k]](self.late)
                    if probe is not None:
                        self.probes[k] = probe
                    self.issued[k] += 1
            self.done.append(jnp.dot(_bf(lhs), rhs, preferred_element_type=F32))
            return self.done[-1]

    def kernel(x_hbm, aqkv_hbm, awo_hbm, bqkv_hbm, bwo_hbm, out_hbm,
               xs, raw, wa, wb, wc, xa, xb, fa, fb, kf, xn_s, q_s, k_s, vt_s, o_s, kv_s, z_s, kz_s,
               m_s, ot_s, on_s, acc_s, kr_s, ka, kb, qa, qb, sem_x, sem_w, *scores):
        X, F = (xa, xb), (fa, fb)
        import contextlib
        sc = (lambda n: jax.named_scope(n)) if cfg.get("PROF") else (lambda n: contextlib.nullcontext())

        def x_copy(i):
            return pltpu.make_async_copy(x_hbm.at[i], xs.at[i], sem_x.at[i])

        def out_copy(i):
            return pltpu.make_async_copy(xs.at[i], out_hbm.at[i], sem_x.at[i])

        def w_copy(p):
            src, c = ((aqkv_hbm, p), (awo_hbm, p - 6), (bqkv_hbm, p - 8), (bwo_hbm, p - 14))[
                (p >= 6) + (p >= 8) + (p >= 14)]
            return pltpu.make_async_copy(src.at[:, :, pl.ds(c * PW, PW)], raw.at[p % 12], sem_w.at[p])

        def start(blocks, panels):
            for copy in [x_copy(i) for i in blocks] + [w_copy(p) for p in panels]:
                copy.start()

        def w_wait(p):
            pltpu.make_async_copy(raw.at[p], raw.at[p], sem_w.at[p]).wait()

        def weight_ops(alg, slot, piece, dst, panel, z, reload=True):
            tile0, rows, packed = (piece >> 3) * 4, _at((piece & 7) * 16, 16), _at(piece * 8, 8)
            def loader(s):
                def quad(i, j):
                    w = raw[s, pl.ds(tile0 + 2 * i, 2), rows, pl.ds(j * 256, 256)].astype(F32)
                    if alg is Classic:
                        return w.reshape(32, 256)
                    return jnp.concatenate([jnp.concatenate(
                        [_mul(w[a, :, b * 128:(b + 1) * 128], _scale(alg.rhs_scale, 2 * i + a, 2 * j + b))
                         for b in (0, 1)], axis=1) for a in (0, 1)])
                return _memo(quad)
            shared = loader(slot)
            def task(m, late):
                dst[panel, m, packed, :] = _leaves(alg.rhs, loader(slot + z * m) if reload else shared, m, late())
                return lambda: dst[panel + z, m, packed, pl.ds(0, 128)]
            return [lambda late, m=m: task(m, late) for m in range(7)]

        def token_ops(alg, src, i, dst, z):
            def piece(r, c):
                quad = _memo(lambda a, b: src[i + z, pl.ds(2 * a, 2), pl.ds(r, 16),
                                              pl.ds(c * 512 + b * 256, 256)].reshape(32, 256))
                def task(m, late):
                    dst[0, m, c, pl.ds(r // 2, 8), :] = _leaves(alg.lhs, quad, m, late())
                    return lambda: dst[z, m, c, pl.ds(r // 2, 8), pl.ds(0, 128)]
                return [lambda late, m=m: task(m, late) for m in range(7)]
            return [t for r in range(0, MB, 16) for c in range(2) for t in piece(r, c)]

        def project(src, p0, emit, pace, mult=1.0):
            alg, w, base = (Balanced, wa, 0) if p0 < 6 else (Classic, wb, 6) if p0 < 14 else (Classic, wc, 14)
            for p in (p0, p0 + 1):
                z = pace.z * (2 * p + 1)
                panel = p - base + z
                def product(m, n):
                    cols = pl.ds(n * 128, 128)
                    return pace.dot(jnp.concatenate([src[z, m, c, :, cols] for c in range(2)], axis=1),
                                    _bf(w[panel, m, :, cols]))
                _combine(alg, product, lambda mi, nj, v: emit(
                    mi, 4 * (p - p0) + nj, _mul(v, mult * _scale(alg.out_scale, mi, nj))))

        def layer_norm(alg, i, dst, z):
            def task(r, late):
                x, token = xs[i, pl.ds(r, 8), :].astype(F32), late()
                if token is not None:
                    x = jnp.concatenate([_after(x[:, :128], token), x[:, 128:]], axis=1)
                xc, rs = _centered(x)
                if alg is not Classic:
                    scaled = _memo(lambda s: jnp.broadcast_to(_mul(rs, s), (8, 128)))
                    rs = jnp.concatenate([scaled(_scale(alg.lhs_scale, r // MB, g % 4)) for g in range(G)], axis=1)
                dst[0, r // MB, pl.ds(r % MB, 8), :] = xc * rs
                return lambda: pltpu.bitcast(dst[z, r // MB, pl.ds(r % MB, 8), pl.ds(0, 128)], U32)
            return [lambda late, r=r: task(r, late) for r in range(0, TM, 8)]

        def to_f32(dst, i):
            def emit(mi, g, v):
                dst[i, mi, :, pl.ds(g * 128, 128)] = v
            return emit

        def to_bf16(dst, i):
            def emit(mi, g, v):
                dst[g, i, pl.ds(mi * MB // 2, MB // 2), :] = _pack(v)
            return emit

        def to_transposed(dst, i):
            hold = {}
            def emit(mi, g, v):
                hold[mi, g] = v
                if (mi ^ 1, g) in hold:
                    both = jnp.concatenate([hold.pop((mi & 2, g)), hold.pop((mi | 1, g))])
                    dst[g, i, pl.ds(0, 64), pl.ds((mi & 2) * MB, 2 * MB)] = pltpu.bitcast(both.astype(BF).T, U32)
            return emit

        def to_residual(i):
            def emit(mi, g, v):
                r, c = pl.ds(mi * MB, MB), pl.ds(g * 128, 128)
                xs[i, r, c] = (xs[i, r, c].astype(F32) + v).astype(BF)
            return emit

        def output_phase(z0, p0, stage, alg_next, pending=()):
            done = []
            for i in range(NB):
                u, z = i % 2, z0 << i
                if stage is not None or i == NB - 1:
                    lists = [token_ops(alg_next if i == NB - 1 else Classic, F[1 - u], 0, X[1 - u], z)]
                else:
                    lists = [token_ops(Classic, o_s, i + 1, X[1 - u], z)]
                norm = i >= (3 if stage is None else NB - 2)
                if stage is None and norm:
                    tasks = layer_norm(alg_next, 0, fa, z) + layer_norm(alg_next, 1, fb, z)
                    lists.append(tasks[(i - 3) * 15:(i - 2) * 15])
                elif norm:
                    lists.append(layer_norm(alg_next, u, F[u], z))
                elif stage is not None:
                    lists.append(stage(i + 2, F[u], z))
                else:
                    lists.append(_part(pending, i, 3))
                project(X[u], p0, to_residual(i),
                        Pacer(z, done, 2 * NP, [(t, 0, 90) for t in lists], cfg["LW"] if norm else cfg["WIN2"]))
                if stage is None:
                    out_copy(i).start()

        def features(src, i, use, finish=None):
            vals, out = {}, []
            def feat(g, b, late):
                token = late()
                vals[g, b] = _phi(_after(src[i, b, :, pl.ds(g * 128, 128)],
                                         None if token is None else jnp.tile(token, (MB // 8, 1))))
                return lambda: pltpu.bitcast(vals[g, b][-8:], U32)
            for g in range(G + 1):
                f = [lambda late, g=g, b=b: feat(g, b, late) for b in range(4)] if g < G else []
                if g:
                    f.insert(cfg["MP"], lambda late, g=g - 1: use(g, [vals[g, b] for b in range(4)]))
                    if finish is not None:
                        f.append(lambda late, g=g - 1: finish(g))
                out += f
            return out

        def lin_accumulate(i, k_src, k_index):
            def use(g, pk):
                z_s[g] += sum(jnp.sum(p.reshape(MB // 8, 8, 128), axis=0) for p in pk)
                kv_s[g] += jnp.dot(_bf(vt_s[g, i]), jnp.concatenate(pk).astype(BF), preferred_element_type=F32)
            return features(k_src, k_index, use)

        def lin_finalize():
            def task(g):
                row = lax.broadcasted_iota(jnp.int32, (128, 128), 0)
                head = lax.broadcasted_iota(jnp.int32, (128, 128), 1) >> 5
                kz_s[g, :64, :] = _pack(jnp.where((row >> 5) == head, kv_s[g], 0.0))
                zsum = jnp.broadcast_to(jnp.sum(z_s[g], axis=0, keepdims=True), (16, 128))
                kz_s[g, 64:, :] = _pack(jnp.where(row[:16] == head[:16], zsum, 0.0))
                kv_s[g] = jnp.zeros((128, 128), F32)
                z_s[g] = jnp.zeros((8, 128), F32)
            return [lambda late, g=g: task(g) for g in range(G)]

        def lin_output(i, dst, z):
            numden = {}
            def use(g, pq):
                numden[g] = lax.dot_general(_bf(kz_s[g + z]), jnp.concatenate(pq).astype(BF),
                                            (((1,), (1,)), ((), ())), preferred_element_type=F32)
            def finish(g):
                nd = numden.pop(g)
                inv = 1.0 / (nd[128:136] + 1e-6)
                o = jnp.concatenate([nd[h * DH:(h + 1) * DH] * inv[h:h + 1] for h in range(4)])
                dst[0, :, :, pl.ds(g * 128, 128)] = o.T.reshape(4, MB, 128)
            return features(o_s, i, use, finish)

        def lin_phase(rep, z0):
            def panel_ops(slot, panel, z):
                return [t for r in range(16) for t in weight_ops(Classic, slot, r, wb, panel, z)]

            def keys_values(i, u, pace):
                project(X[u], 4, to_transposed(vt_s, i), pace)
                project(X[u], 2, to_f32(kf, 0), pace)

            def body(it, z):
                @pl.when(rep == 0)
                def _():
                    for i in (2 * it, 2 * it + 1):
                        x_copy(i + 2).wait()
                        w_wait(6 + i)

                pl.when((rep == 0) & (it == NB // 2 - 2))(lambda: start((), (6, 7, 12, 13)))
                done = []
                for u in range(2):
                    i, zu = 2 * it + u, z << u
                    pace = Pacer(zu, done, 6 * NP, [
                        (panel_ops(6 + i, i, zu), 0, cfg["W1"]),
                        (token_ops(Balanced, F[1 - u], 0, X[1 - u], zu), 0, cfg["O1"]),
                        (lin_accumulate(i + zu, kf, zu), cfg["A0"], cfg["A1"]),
                        (layer_norm(Balanced, i + 2, F[u], zu), 0, cfg["L1"])], cfg["WIN1"])
                    keys_values(i, u, pace)
                    project(X[u], 0, to_f32(o_s, i), pace)
                return z
            with sc("P1loop"):
                lax.fori_loop(1 - rep, NB // 2 - 1, body, z0)
            if cfg.get("NOPEEL"):
                return

            @pl.when(rep == 0)
            def _():
                for p in (6, 7, 12, 13):
                    w_copy(p).wait()
                start((), (14, 15))

            @pl.when(rep == 1)
            def _():
                for i in range(NB):
                    out_copy(i).wait()
            done, (za, zb) = [], (z0 << NB, z0 << (NB + 1))
            ops = panel_ops(6, 0, za) + panel_ops(7, 1, za) + panel_ops(0, 6, zb) + panel_ops(1, 7, zb)
            a, b, c = (len(ops) * cfg[k] // 100 for k in ("C0", "C1", "C2"))
            keys_values(NB - 2, 0, Pacer(za, done, 4 * NP, [
                (ops[:a], 0, 100), (token_ops(Balanced, fb, 0, xb, za), 0, 92)], cfg["WIN1"]))
            keys_values(NB - 1, 1, Pacer(zb, done, 4 * NP, [
                (ops[a:b], 0, 100), (lin_accumulate(NB - 2, kf, za), 3, 50)], cfg["WIN1"]))
            for u, z, tasks, more in (
                    (0, za, lin_accumulate(NB - 1 + zb, kf, zb) + lin_finalize() + lin_output(0, fa, za), ops[b:c]),
                    (1, zb, lin_output(1, fb, zb), ops[c:])):
                lists = [(more, 0, 100), (tasks, 6 * (1 - u), 95)] + [(token_ops(Classic, fa, 0, xa, z), 5, 92)] * u
                project(X[u], 0, to_f32(o_s, NB - 2 + u), Pacer(z, done, 2 * NP, lists, cfg["WIN2"]))

        def qkv_phase(z0):
            def body(it, zc):
                done = []
                for u in range(2):
                    i, z = 2 * it + u, zc << u
                    pace = Pacer(z, done, 6 * NP, [
                        (token_ops(Classic, F[1 - u], 0, X[1 - u], z), 0, 90),
                        (layer_norm(Classic, jnp.minimum(i + 2, NB - 1), F[u], z), 0, 90),
                        ([t for r in range(4) for t in weight_ops(Classic, 2 + (i >> 2), (i & 3) * 4 + r, wc, i >> 2, z)],
                         0, 95)], cfg["WIN3"])
                    project(X[u], 12, to_transposed(vt_s, i), pace)
                    project(X[u], 8, to_transposed(q_s, i), pace, QSCALE)
                    project(X[u], 10, to_bf16(k_s, i), pace)
                return zc
            lax.fori_loop(0, NB // 2, body, z0)

        def q_rows(g, j, rows):
            return jnp.concatenate([q_s[g, j * (BQ // TM) + b, rows, :] for b in range(BQ // TM)], axis=1)

        def widen_q(g, head, j, token=None):
            q = q_rows(g, j, _at(head * (DH // 2), DH // 2))
            q = _bf(q if token is None else q | jnp.tile(token, (DH // 16, BQ // 128))).astype(F32)
            q = jnp.concatenate([q, q[:8]])
            for b in range(BQ // 128):
                (qa, qb)[j % 2][0, b] = q[:, b * 128:(b + 1) * 128]

        def spread_k(g, pair, u, z):
            def skew(late):
                ends = [(c + 1) * CK for c in VPU]
                k = jnp.concatenate([k_s[g, (e - RG) // TM, pl.ds((e - RG) % TM // 2, RG // 2), :] for e in ends])
                token = late()
                k = _bf(k if token is None else k | jnp.tile(token, (len(VPU), 1))).astype(F32)
                left = lambda v, n: jnp.concatenate([v[:, n:], v[:, :n]], axis=1)
                row = lax.broadcasted_iota(jnp.int32, k.shape, 0)
                lane = lax.broadcasted_iota(jnp.int32, k.shape, 1) & (DH - 1)
                k = jnp.where(pair == 0, k, left(k, 2 * DH))
                for n in (1, 2, 4):
                    k = jnp.where((row & n) == 0, k, jnp.where(lane < DH - n, left(k, n), left(k, 128 - DH + n)))
                kr_s[u] = pltpu.bitcast(k, U32)
            def task(d0, late):
                k, token = kr_s[u + z * d0], late()
                if token is not None:
                    k = k | jnp.tile(token, (2 * len(VPU), 1))
                for d in range(d0, d0 + cfg["KD"]):
                    column = jnp.broadcast_to(k[:, u * DH + d:u * DH + d + 1], k.shape)
                    (ka, kb)[u][0, d] = column.reshape(-1, 8, 128)
            return [skew, lambda late: None] + [lambda late, d=d: task(d, late) for d in range(0, DH, cfg["KD"])]

        def stream(qk, c0, c1, pv, m, mx, z, extra, shared):
            steps, tiles = CK // RG, BQ // 128
            ms, mxu_scores, probs = [m], {}, {}
            st = dict(mx=mx, token=None, acc=None, l=None, stored=c0 * steps, d=0)
            zs, zero, nothing = _memo(lambda k: z * k), _zero_tile(z), jnp.zeros((8, 128), U32)
            head_rows = _memo(lambda t, h: _at(jnp.where(qk[t][1] == h // 2, h * (DH // 2), 64), DH // 2))

            def score_ref(j, row):
                return scores[j % 2 * NS + row // (S // NS)], row % (S // NS) // 8

            def score(ci):
                t, c = divmod(ci, NC)
                g, _, u, j = qk[t]
                keys = CK - RG if ci < shared and c in VPU else CK
                k = k_s[g + zs(t + 1), c * CK // TM, pl.ds(c * CK % TM // 2, keys // 2), :]
                gq = g + zs(c + 1)
                q = {h: q_rows(gq, j, head_rows(t, h)) for h in (u, u + 2)}
                q = jnp.concatenate([q[h] if h in q else jnp.zeros_like(q[u]) for h in range(4)])
                mxu_scores[ci] = jnp.dot(_bf(k), _bf(q), preferred_element_type=F32)

            def vpu_terms(ci, upto, token):
                t, c = divmod(ci, NC)
                while st["d"] < upto:
                    d = st["d"]
                    st["d"] += 1
                    k = (ka, kb)[qk[t][2]][zs(t + 1), d, pl.ds(VPU.index(c) * 2, 2)]
                    k = pltpu.bitcast(k if token is None else k | token, F32)
                    term = k[:, None] * (qa, qb)[qk[t][3] % 2][pl.ds(zs(c + 1), 1), :, pl.ds(d, 8), :]
                    st["vpu"] = term if d == 0 else st["vpu"] + term

            def store_scores(upto):
                while st["stored"] < min(upto, c1 * steps):
                    ci, k = divmod(st["stored"], steps)
                    st["stored"] += 1
                    t, c = divmod(ci, NC)
                    if ci < shared:
                        ahead = min((v - c) % NC for v in VPU)
                        behind = min((c - v - 1) % NC for v in VPU)
                        if (behind, k) == (0, 0):
                            st["d"] = 0
                        vpu_terms(ci + ahead, (behind * steps + k + 1) * DH // ((behind + ahead + 1) * steps), st["token"])
                    for r in range(k * RG, (k + 1) * RG, 8):
                        if r < mxu_scores[ci].shape[0]:
                            s = mxu_scores[ci][r:r + 8]
                        else:
                            s = jnp.concatenate([st["vpu"][r % RG // 8, b] for b in range(tiles)], axis=1)
                        ref, row = score_ref(qk[t][3], c * CK + r)
                        ref[0, row] = s
                        st["mx"] = s if st["mx"] is None else jnp.maximum(st["mx"], s)
                    st["token"] = pltpu.bitcast(s[:, :128], U32) & zero
                    if (c, k) == (NC - 1, steps - 1):
                        top = jnp.broadcast_to(jnp.max(st["mx"], axis=0, keepdims=True), (8, BQ))
                        ms.append(pltpu.bitcast(top, U32)[None])
                        st["mx"] = None

            def exponentiate(ci, token=None):
                t, c = divmod(ci, NC)
                parts = {}
                for k in reversed(range(steps)):
                    store_scores((ci + c0) * steps - k - cfg["LEAD"])
                    if ci < c1 - c0:
                        token = st["token"]
                    if token is not None:
                        every = ci >= c1 - c0 or (c, k) == (0, steps - 1)
                        ms[t] = ms[t] | jnp.concatenate(
                            [token if every or (b + k + 1) % cfg["HG"] == 0 else nothing for b in range(tiles)], axis=1)
                        token = None
                    ref, row = score_ref(pv[t][3], c * CK + k * RG)
                    parts[k] = jnp.exp2(ref[z, pl.ds(row, RG // 8)] - pltpu.bitcast(ms[t], F32))
                    part = jnp.sum(parts[k], axis=0)
                    st["l"] = part if st["l"] is None else st["l"] + part
                probs[ci] = jnp.concatenate([parts[k] for k in range(steps)]).reshape(CK, BQ).astype(BF)

            def weigh(ci):
                t, c = divmod(ci, NC)
                g, pair, u, j = pv[t]
                v = vt_s[g + zs(t + 1), c * CK // TM, _at(pair * DH + u * (DH // 2), DH // 2), pl.ds(c * CK % TM, CK)]
                o = jnp.dot(_bf(v), probs.pop(ci), preferred_element_type=F32)
                if c:
                    o = acc_s[z] + o
                elif st["acc"] is not None:
                    o = st["acc"] + o
                if c < NC - 1:
                    acc_s[0] = o
                else:
                    ot_s[u, j, :DH, :] = o
                    ot_s[u, j, DH:, :] = st["l"]
                    st["acc"] = pltpu.bitcast(pltpu.bitcast(o, jnp.int32) & z, F32)
                    st["l"] = None

            for ci in range(c0, c1):
                if ci < shared and ci % NC == NC - 6:
                    g, pair, u, j = qk[ci // NC + 1]
                    widen_q(g, 2 * pair + u, j, st["token"])
                for tasks, first, end in extra:
                    if first <= ci < end:
                        for task in _part(tasks, ci - first, end - first):
                            task(lambda: st["token"])
                score(ci)
                if pv:
                    exponentiate(ci - c0)
                    weigh(ci - c0)
            store_scores(c1 * steps)
            if st["mx"] is not None:
                m_s[0] = ms[-1][0]
                m_s[1] = pltpu.bitcast(st["mx"], U32)
            return [lambda late, n=n: (exponentiate(n, late()), weigh(n))[1] for n in range(c1 - c0, len(pv) * NC)]

        def normalize(slot, pair, u, j):
            def task(late):
                token = late()
                l = _after(ot_s[u, j, DH:, :], None if token is None else jnp.tile(token, (1, BQ // 128)))
                on_s[slot, j, _at((2 * pair + u) * DH, DH), :] = (
                    ot_s[u, j, :DH, :] * (1.0 / jnp.sum(l, axis=0, keepdims=True)))
            return [task]

        def transpose_out(slot, g, j):
            def task(b, late):
                o = on_s[slot, j, :, pl.ds(b * 128, 128)]
                o = jnp.concatenate([_after(o[:8], late()), o[8:]])
                o_s[2 * j + b // 2, pl.ds(b % 2 * 2, 2), :, _at(g * 128, 128)] = o.T.reshape(2, MB, 128)
            return [lambda late, b=b: task(b, late) for b in range(BQ // 128)]

        def attention(z0):
            widen_q(0, 0, 1)
            stream([(0, 0, 0, 0), (0, 0, 0, 1)], 0, NC + 2, [], None, None, z0, [(spread_k(0, 0, 0, z0), 0, NC)], 0)

            def finish(j):
                return normalize(1, 1, 0, j) + normalize(1, 1, 1, j) + transpose_out(1, G - 1, j)

            def body(it, z, last=False):
                g, pair, m, mx = it >> 1, it & 1, m_s[:1], pltpu.bitcast(m_s[1], F32)
                items = [(g, pair, u, j) for u in range(2) for j in range(NQ)]
                prev = g - 1 if last else jnp.maximum(g - 1, 0)
                extra = [([t for u in range(2) for j in range(NQ)
                           for t in normalize(((it + 3) >> 1) & 1, 1 - pair, u, j)], 4, 12),
                         (spread_k(g, pair, 1, z), 8, 3 * NC - 4),
                         (transpose_out(1 - (g & 1), prev, 2 * pair) + transpose_out(1 - (g & 1), prev, 2 * pair + 1),
                          *((3 * NC, 5 * NC) if last else (cfg["E1"], 8 * NC - 6)))]
                if last:
                    extra.append((finish(0), 5 * NC + 3, 5 * NC + 9))
                    extra.append((token_ops(Classic, o_s, 0, xa, z), 5 * NC + 11, 7 * NC - 2))
                    return stream(items[1:], 2, 7 * NC, items, m, mx, z, extra, 5 * NC + 2)
                g, pair = (it + 1) >> 1, (it + 1) & 1
                extra.append((spread_k(g, pair, 0, z), 3 * NC, cfg["E1"]))
                stream(items[1:] + [(g, pair, 0, 0), (g, pair, 0, 1)], 2, 8 * NC + 2, items, m, mx, z, extra,
                       8 * NC + 2)
                return z
            with sc("P4loop"):
                lax.fori_loop(0, 2 * G - 1, body, z0)
            if "5" not in PH:
                return []
            return finish(1) + body(2 * G - 1, z0, True) + finish(2) + finish(3)

        def first_norm(i):
            def body(n, c):
                for r in range(0, TM // 2, 16):
                    xc, rs = _centered(xs[i, _at(n * (TM // 2) + r, 16), :].astype(F32))
                    xn_s[0, 2 * i + n, pl.ds(r // 2, 8), :] = _pack(xc * rs)
                return c
            lax.fori_loop(0, 2, body, 0)

        def first_panel(p, z, done, lists):
            tasks = [t for r in range(16) for t in weight_ops(Balanced, p, r, wa, p, z, False)]
            pace = Pacer(z, done, 64, [(tasks, 0, cfg["S1"])] + lists, cfg["WIN0"], cfg["DY0"])
            for nj in range(4):
                for b in range(4):
                    zx, slot, total = z * (nj + 1), p + z * (b + 8), None
                    for k in range(4):
                        part = pace.dot(xn_s[zx, b, :, pl.ds(k * 256, 256)],
                                        raw[slot, pl.ds(2 * k, 2), :, pl.ds(nj * 128, 128)].reshape(256, 128))
                        total = part if total is None else total + part
                    o_s[(p >> 1) * 2 + b // 2, pl.ds(b % 2 * 2, 2), :, _at((p & 1) * PW + nj * 128, 128)] = (
                        total.reshape(2, MB, 128))

        def first_v(i):
            def task(g, late):
                v = o_s[4 + i, :, :, pl.ds(g * 128, 128)].reshape(TM, 128)
                v = jnp.concatenate([_after(v[:8], late()), v[8:]])
                vt_s[g, i] = pltpu.bitcast(v.astype(BF).T, U32)
            return [lambda late, g=g: task(g, late) for g in range(G)]

        if cfg.get("NOST"):
            first_panel = lambda *a: None
        start((0, 1), ())
        kv_s[...] = jnp.zeros_like(kv_s)
        z_s[...] = jnp.zeros_like(z_s)
        ot_s[...] = jnp.ones_like(ot_s)
        on_s[1, :, :64, :] = jnp.zeros((NQ, 64, BQ), F32)
        q_s[:, :, 64:, :] = jnp.zeros((G, NB, 16, TM), U32)
        for i in range(2):
            x_copy(i).wait()
            start((), (2,)[i:])
            first_norm(i)

        def kv_panel(p, c):
            w_wait(p)
            for n, nxt in enumerate((((), (3, 4)), ((), (5, 0)), ((2, 3), (1,)), ((4, 5), (8,)))):
                pl.when(p == 2 + n)(lambda nxt=nxt: start(*nxt))
            first_panel(p, p >> 3, [], [])
            return p >> 3
        with sc("S0"):
            zero = lax.fori_loop(2, 6, kv_panel, 0)
        for copy in (x_copy(2), x_copy(3), w_copy(0), w_copy(1)):
            copy.wait()
        start((), (9, 10))
        finished = []
        with sc("S1"):
            for u in range(2):
                first_panel(u, zero << 4 * u, finished, [
                    (layer_norm(Balanced, 2 + u, F[u], zero), 0, cfg["H0"]),
                    (token_ops(Balanced, fa, 0, xa, zero), 0, 94) if u else (first_v(0) + first_v(1), 0, cfg["H0"]),
                    (lin_accumulate(u, o_s, 2 + u), cfg["H0"], 97)])
        start((6, 7), (11,))

        def layer_pair(rep, c):
            z0 = rep >> 1
            if "1" in PH:
                with sc("P1"):
                    lin_phase(rep, z0)
            if "2" in PH:
                with sc("P2"):
                    if cfg["SP"]:
                        lax.fori_loop(z0, 1, lambda z, c: output_phase(z, 6, lin_output, Classic), None)
                    else:
                        output_phase(z0, 6, lin_output, Classic)

            @pl.when(rep == 0)
            def _():
                w_copy(14).wait()
                w_copy(15).wait()
            if "3" in PH:
                with sc("P3"):
                    qkv_phase(z0)
            rest = ()
            if "4" in PH:
                with sc("P4"):
                    rest = attention(z0)
            if "5" in PH:
                with sc("P5"):
                    output_phase(z0, 14, None, Balanced, rest)
            if len(PH) < 5:
                u = (q_s[rep, rep, :8, :128] | k_s[rep, rep, :8] | vt_s[rep, rep, :8, :128] | wb[rep, rep, :8, :128]
                     | wa[rep, rep, :8, :128] | wc[rep, rep, :8, :128] | xa[0, rep, rep, :8, :128])
                f = (pltpu.bitcast(u, F32) + kv_s[rep, :8] + z_s[rep] + o_s[rep, rep, :8, :128]
                     + fa[0, rep, :8, :128] + fb[0, rep, :8, :128])
                xs[0, :8, :128] = f.astype(BF)
            return c
        lax.fori_loop(0, 2, layer_pair, 0)
        for i in range(NB):
            out_copy(i).wait()

    any_spec = pl.BlockSpec(memory_space=pl.ANY)
    return pl.pallas_call(
        kernel,
        out_shape=jax.ShapeDtypeStruct((NB, TM, D), BF),
        in_specs=[any_spec] * 5,
        out_specs=any_spec,
        scratch_shapes=[
            pltpu.VMEM((NB, TM, D), BF),
            pltpu.VMEM((12, G, 128, PW), BF),
            pltpu.VMEM((6, 7, 128, 7 * 128), U32),
            pltpu.VMEM((8, 7, 128, 7 * 128), U32),
            pltpu.VMEM((2, 7, 128, 7 * 128), U32),
            pltpu.VMEM((1, 7, 2, MB // 2, 7 * 128), U32),
            pltpu.VMEM((1, 7, 2, MB // 2, 7 * 128), U32),
            pltpu.VMEM((1, 4, MB, D), F32),
            pltpu.VMEM((1, 4, MB, D), F32),
            pltpu.VMEM((1, 4, MB, D), F32),
            pltpu.VMEM((1, 4, 64, D), U32),
            pltpu.VMEM((G, NB, 80, TM), U32),
            pltpu.VMEM((G, NB, TM // 2, 128), U32),
            pltpu.VMEM((G, NB, 64, TM), U32),
            pltpu.VMEM((NB, 4, MB, D), F32),
            pltpu.VMEM((G, 128, 128), F32),
            pltpu.VMEM((G, 8, 128), F32),
            pltpu.VMEM((G, 72, 128), U32),
            pltpu.VMEM((2, 8, BQ), U32),
            pltpu.VMEM((2, NQ, DH + 8, BQ), F32),
            pltpu.VMEM((2, NQ, 128, BQ), F32),
            pltpu.VMEM((1, DH, BQ), F32),
            pltpu.VMEM((2, RG * len(VPU), 128), U32),
            pltpu.VMEM((1, DH, 2 * len(VPU), 8, 128), U32),
            pltpu.VMEM((1, DH, 2 * len(VPU), 8, 128), U32),
            pltpu.VMEM((1, BQ // 128, DH + 8, 128), F32),
            pltpu.VMEM((1, BQ // 128, DH + 8, 128), F32),
            pltpu.SemaphoreType.DMA((NB,)),
            pltpu.SemaphoreType.DMA((16,)),
        ] + [pltpu.VMEM((1, S // NS // 8, 8, BQ), F32)] * (2 * NS),
        compiler_params=pltpu.CompilerParams(vmem_limit_bytes=122 * 2 ** 20),
        interpret=cfg.get("INTERP", False),
    )


@jax.jit
def pallas_interleave_layers__linear_attn_block__mha_block__prompt_kernel(
    A_x: jax.Array,
    A_wqkv: jax.Array,
    A_wo: jax.Array,
    B_x: jax.Array,
    B_wqkv: jax.Array,
    B_wo: jax.Array,
):
    del B_x
    weights = [w.reshape(G, 128, -1) for w in (A_wqkv, A_wo, B_wqkv, B_wo)]
    return build(CFG)(A_x.reshape(NB, TM, D), *weights).reshape(A_x.shape)
```

```python
import math

import jax
import jax.numpy as jnp
from jax import lax
import jax.experimental.pallas as pl
import jax.experimental.pallas.tpu as pltpu

S, D, DH = 2048, 1024, 32
G = D // 128
TM = 256
NB = S // TM
MB = TM // 4
NP = 49
PW = 512
BQ, CK, RG = 512, 128, 16
NQ, NC = S // BQ, S // CK
NS = 4
VP = 4
NV = NC // VP
QSCALE = DH ** -0.5 * math.log2(math.e)
U32, BF, F32 = jnp.uint32, jnp.bfloat16, jnp.float32


class Classic:
    lhs_scale = rhs_scale = out_scale = ((1.0, 1.0), (1.0, 1.0))
    lhs = (lambda q: q(1, 0) - q(0, 0), lambda q: q(1, 0) + q(1, 1), lambda q: q(1, 1),
           lambda q: q(0, 1) - q(1, 1), lambda q: q(0, 0) + q(1, 1), lambda q: q(0, 0) + q(0, 1),
           lambda q: q(0, 0))
    rhs = (lambda q: q(0, 0) + q(0, 1), lambda q: q(0, 0), lambda q: q(1, 0) - q(0, 0),
           lambda q: q(1, 0) + q(1, 1), lambda q: q(0, 0) + q(1, 1), lambda q: q(1, 1),
           lambda q: q(0, 1) - q(1, 1))

    @staticmethod
    def step(m, v, a, emit):
        if m == 0:
            a["d"] = v
        elif m == 1:
            a["d"] = a["d"] - v
            a["c"] = v
        elif m == 2:
            emit(1, 0, a["c"] + v)
            a["c"] = v
        elif m == 3:
            a["c"] = a["c"] + v
        elif m == 4:
            a["c"] = a["c"] + v
            a["d"] = a["d"] + v
        elif m == 5:
            emit(0, 0, a["c"] - v)
            a["c"] = v
        else:
            emit(0, 1, a["c"] + v)
            emit(1, 1, a["d"] + v)


def _diag(q):
    return q(0, 0) + q(1, 1)


class Balanced:
    lhs_scale = ((0.5, 0.25), (1.0, 0.5))
    rhs_scale = ((1.0, 0.5), (2.0, 1.0))
    out_scale = ((1.0, 2.0), (0.5, 1.0))
    lhs = (lambda q: q(0, 0) + q(0, 1), lambda q: q(0, 0) - q(0, 1), _diag,
           lambda q: q(1, 1) - q(0, 1), lambda q: q(1, 1) + q(0, 1),
           lambda q: _diag(q) + (q(0, 1) + q(1, 0)), lambda q: _diag(q) - (q(0, 1) + q(1, 0)))
    rhs = (lhs[4], lhs[3], lambda q: 2.0 * _diag(q), lhs[5], lhs[6], lhs[1], lhs[0])

    @staticmethod
    def step(m, v, a, emit):
        if m == 0:
            a["p"] = v
        elif m == 1:
            a["s"] = a["p"] + v
            a["d"] = a["p"] - v
            emit(0, 1, a["d"])
        elif m == 2:
            a["t"] = v - a["s"]
        elif m in (3, 5):
            a["c"] = a["t"] - v
            a["d"] = a["d"] + v
        elif m == 4:
            emit(0, 0, a["c"] - v)
            a["d"] = a["d"] - v
        else:
            emit(1, 1, a["c"] - v)
            emit(1, 0, a["d"] - v)


def _scale(table, i, j):
    return table[i >> 1][j >> 1] * table[i & 1][j & 1]


def _mul(v, s):
    return v if s == 1.0 else v * s


def _memo(f):
    seen = {}

    def g(*key):
        if key not in seen:
            seen[key] = f(*key)
        return seen[key]
    return g


def _after(v, token):
    return v if token is None else pltpu.bitcast(pltpu.bitcast(v, U32) | token, F32)


def _pack(v):
    return pltpu.bitcast(v.astype(BF), U32)


def _bf(v):
    return pltpu.bitcast(v, BF)


def _leaves(forms, quad, m, token):
    top = forms[m](quad)

    @_memo
    def tile(i, j):
        r, c = 16 * i, slice(128 * j, 128 * j + 128)
        if i != j or token is None:
            return top[r:r + 16, c]
        return jnp.concatenate([_after(top[r:r + 8, c], token), top[r + 8:r + 16, c]])
    return _pack(jnp.concatenate([f(tile) for f in forms], axis=1))


def _combine(alg, product, emit):
    outer = {}
    for m in range(7):
        def inner(i, j, v, m=m):
            alg.step(m, v, outer.setdefault((i, j), {}), lambda a, b, r: emit(2 * a + i, 2 * b + j, r))
        acc = {}
        for n in range(7):
            alg.step(n, product(m, n), acc, inner)


def _phi(t):
    return jnp.where(t > 0, t + 1.0, jnp.exp(t)) + 1e-6


def _centered(x):
    xc = x - jnp.mean(x, axis=-1, keepdims=True)
    return xc, lax.rsqrt(jnp.mean(xc * xc, axis=-1, keepdims=True) + 1e-5)


def _at(start, n):
    return pl.ds(start if isinstance(start, int) else pl.multiple_of(start, n), n)


def _zero_tile(z):
    return jnp.full((8, 128), z, jnp.int32).astype(U32)


def _part(tasks, i, n):
    return tasks[i * len(tasks) // n:(i + 1) * len(tasks) // n]


class Pacer:
    def __init__(self, z, done, n, lists, window, delay, every):
        self.z, self.zero, self.done = z, _zero_tile(z), done
        self.window, self.delay, self.every = window, delay, every
        self.lists = [(t, max(n * a // 100, 0 if done else 1), n * b // 100) for t, a, b in lists]
        self.t, self.issued, self.probes, self.due = 0, [0] * len(lists), {}, {}
        self.token = _memo(lambda i: pltpu.bitcast(done[i][:8], U32) & self.zero)

    def late(self):
        return self.token(max(0, len(self.done) - self.window)) if self.done else None

    def dot(self, lhs, rhs):
        if self.probes and self.t % self.every == 0:
            token = self.zero
            for probe in self.probes.values():
                token = token & probe()
            self.probes = {}
            self.due[self.t + self.delay] = token
        if self.t in self.due:
            lhs = jnp.concatenate([lhs[:8] | jnp.tile(self.due.pop(self.t), (1, 2)), lhs[8:]])
        self.t += 1
        for k, (tasks, a, b) in enumerate(self.lists):
            while self.issued[k] < min(len(tasks), (self.t - a) * len(tasks) // (b - a)):
                probe = tasks[self.issued[k]](self.late)
                if probe is not None:
                    self.probes[k] = probe
                self.issued[k] += 1
        self.done.append(jnp.dot(_bf(lhs), rhs, preferred_element_type=F32))
        return self.done[-1]


def _kernel(x_hbm, aqkv_hbm, awo_hbm, bqkv_hbm, bwo_hbm, out_hbm,
            xs, raw, wa, wb, wc, xa, xb, fa, fb, kf, xn_s, q_s, k_s, vt_s, o_s, kv_s, z_s, kz_s,
            m_s, ot_s, on_s, acc_s, kr_s, ka, kb, qa, qb, sem_x, sem_w, sem_o, *scores):
    X, F = (xa, xb), (fa, fb)

    def x_copy(i):
        return pltpu.make_async_copy(x_hbm.at[i], xs.at[i], sem_x.at[i])

    def out_copy(n):
        i, c = n // 4, pl.ds(n % 4 * 256, 256)
        return pltpu.make_async_copy(xs.at[i, :, c], out_hbm.at[i, :, c], sem_o.at[n])

    def w_copy(p):
        src, c = ((aqkv_hbm, p), (awo_hbm, p - 6), (bqkv_hbm, p - 8), (bwo_hbm, p - 14))[
            (p >= 6) + (p >= 8) + (p >= 14)]
        return pltpu.make_async_copy(src.at[:, :, pl.ds(c * PW, PW)], raw.at[p % 12], sem_w.at[p])

    def w_wait(p):
        pltpu.make_async_copy(raw.at[p], raw.at[p], sem_w.at[p]).wait()

    def start(blocks, panels):
        for copy in [x_copy(i) for i in blocks] + [w_copy(p) for p in panels]:
            copy.start()

    def weight_ops(alg, slot, piece, dst, panel, z, reload=True):
        tile0, rows, packed = (piece >> 3) * 4, _at((piece & 7) * 16, 16), _at(piece * 8, 8)

        def loader(s):
            def quad(i, j):
                w = raw[s, pl.ds(tile0 + 2 * i, 2), rows, pl.ds(j * 256, 256)].astype(F32)
                if alg is Classic:
                    return w.reshape(32, 256)
                return jnp.concatenate([jnp.concatenate(
                    [_mul(w[a, :, b * 128:(b + 1) * 128], _scale(alg.rhs_scale, 2 * i + a, 2 * j + b))
                     for b in (0, 1)], axis=1) for a in (0, 1)])
            return _memo(quad)
        shared = loader(slot)

        def task(m, late):
            dst[panel, m, packed, :] = _leaves(alg.rhs, loader(slot + z * m) if reload else shared, m, late())
            return lambda: dst[panel + z, m, packed, pl.ds(0, 128)]
        return [lambda late, m=m: task(m, late) for m in range(7)]

    def token_ops(alg, src, i, dst, z):
        def piece(r, c):
            quad = _memo(lambda a, b: src[i + z, pl.ds(2 * a, 2), pl.ds(r, 16),
                                          pl.ds(c * 512 + b * 256, 256)].reshape(32, 256))

            def task(m, late):
                dst[0, m, c, pl.ds(r // 2, 8), :] = _leaves(alg.lhs, quad, m, late())
                return lambda: dst[z, m, c, pl.ds(r // 2, 8), pl.ds(0, 128)]
            return [lambda late, m=m: task(m, late) for m in range(7)]
        return [t for r in range(0, MB, 16) for c in range(2) for t in piece(r, c)]

    def project(src, p0, emit, pace, mult=1.0):
        alg, w, base = (Balanced, wa, 0) if p0 < 6 else (Classic, wb, 6) if p0 < 14 else (Classic, wc, 14)
        for p in (p0, p0 + 1):
            z = pace.z * (2 * p + 1)
            panel = p - base + z

            def product(m, n):
                cols = pl.ds(n * 128, 128)
                return pace.dot(jnp.concatenate([src[z, m, c, :, cols] for c in range(2)], axis=1),
                                _bf(w[panel, m, :, cols]))
            _combine(alg, product, lambda mi, nj, v: emit(
                mi, 4 * (p - p0) + nj, _mul(v, mult * _scale(alg.out_scale, mi, nj))))

    def layer_norm(alg, i, dst, z):
        def task(r, late):
            x, token = xs[i, pl.ds(r, 8), :].astype(F32), late()
            if token is not None:
                x = jnp.concatenate([_after(x[:, :128], token), x[:, 128:]], axis=1)
            xc, rs = _centered(x)
            if alg is not Classic:
                scaled = _memo(lambda s: jnp.broadcast_to(_mul(rs, s), (8, 128)))
                rs = jnp.concatenate([scaled(_scale(alg.lhs_scale, r // MB, g % 4)) for g in range(G)], axis=1)
            dst[0, r // MB, pl.ds(r % MB, 8), :] = xc * rs
            return lambda: pltpu.bitcast(dst[z, r // MB, pl.ds(r % MB, 8), pl.ds(0, 128)], U32)
        return [lambda late, r=r: task(r, late) for r in range(0, TM, 8)]

    def to_f32(dst, i):
        def emit(mi, g, v):
            dst[i, mi, :, pl.ds(g * 128, 128)] = v
        return emit

    def to_bf16(dst, i):
        def emit(mi, g, v):
            dst[g, i, pl.ds(mi * MB // 2, MB // 2), :] = _pack(v)
        return emit

    def to_transposed(dst, i):
        hold = {}

        def emit(mi, g, v):
            hold[mi, g] = v
            if (mi ^ 1, g) in hold:
                both = jnp.concatenate([hold.pop((mi & 2, g)), hold.pop((mi | 1, g))])
                dst[g, i, pl.ds(0, 64), pl.ds((mi & 2) * MB, 2 * MB)] = pltpu.bitcast(both.astype(BF).T, U32)
        return emit

    def to_residual(i, store):
        left = [8] * 4

        def emit(mi, g, v):
            r, c = pl.ds(mi * MB, MB), pl.ds(g * 128, 128)
            xs[i, r, c] = (xs[i, r, c].astype(F32) + v).astype(BF)
            left[g // 2] -= 1
            if store and not left[g // 2]:
                out_copy(4 * i + g // 2).start()
        return emit

    def features(src, i, use, finish=None):
        vals, out = {}, []

        def feat(g, b, late):
            token = late()
            vals[g, b] = _phi(_after(src[i, b, :, pl.ds(g * 128, 128)],
                                     None if token is None else jnp.tile(token, (MB // 8, 1))))
            return lambda: pltpu.bitcast(vals[g, b][-8:], U32)
        for g in range(G + 1):
            f = [lambda late, g=g, b=b: feat(g, b, late) for b in range(4)] if g < G else []
            if g:
                f.insert(3, lambda late, g=g - 1: use(g, [vals[g, b] for b in range(4)]))
                if finish is not None:
                    f.append(lambda late, g=g - 1: finish(g))
            out += f
        return out

    def lin_accumulate(i, k_src, k_index):
        def use(g, pk):
            z_s[g] += sum(jnp.sum(p.reshape(MB // 8, 8, 128), axis=0) for p in pk)
            kv_s[g] += jnp.dot(_bf(vt_s[g, i]), jnp.concatenate(pk).astype(BF), preferred_element_type=F32)
        return features(k_src, k_index, use)

    def lin_finalize():
        def task(g):
            row = lax.broadcasted_iota(jnp.int32, (128, 128), 0)
            head = lax.broadcasted_iota(jnp.int32, (128, 128), 1) >> 5
            kz_s[g, :64, :] = _pack(jnp.where((row >> 5) == head, kv_s[g], 0.0))
            zsum = jnp.broadcast_to(jnp.sum(z_s[g], axis=0, keepdims=True), (16, 128))
            kz_s[g, 64:, :] = _pack(jnp.where(row[:16] == head[:16], zsum, 0.0))
            kv_s[g] = jnp.zeros((128, 128), F32)
            z_s[g] = jnp.zeros((8, 128), F32)
        return [lambda late, g=g: task(g) for g in range(G)]

    def lin_output(i, dst, z):
        numden = {}

        def use(g, pq):
            numden[g] = lax.dot_general(_bf(kz_s[g + z]), jnp.concatenate(pq).astype(BF),
                                        (((1,), (1,)), ((), ())), preferred_element_type=F32)

        def finish(g):
            nd = numden.pop(g)
            inv = 1.0 / (nd[128:136] + 1e-6)
            o = jnp.concatenate([nd[h * DH:(h + 1) * DH] * inv[h:h + 1] for h in range(4)])
            dst[0, :, :, pl.ds(g * 128, 128)] = o.T.reshape(4, MB, 128)
        return features(o_s, i, use, finish)

    def lin_qkv(rep, z0):
        def panel_ops(slot, panel, z):
            return [t for r in range(16) for t in weight_ops(Classic, slot, r, wb, panel, z)]

        def keys_values(i, u, pace):
            project(X[u], 4, to_transposed(vt_s, i), pace)
            project(X[u], 2, to_f32(kf, 0), pace)

        def body(it, z):
            @pl.when(rep == 0)
            def _():
                for i in (2 * it, 2 * it + 1):
                    x_copy(i + 2).wait()
                    w_wait(6 + i)

            pl.when((rep == 0) & (it == NB // 2 - 2))(lambda: start((), (6, 7, 12, 13)))
            done = []
            for u in range(2):
                i, zu = 2 * it + u, z << u
                pace = Pacer(zu, done, 6 * NP, [
                    (panel_ops(6 + i, i, zu), 0, 100),
                    (token_ops(Balanced, F[1 - u], 0, X[1 - u], zu), 0, 80),
                    (lin_accumulate(i + zu, kf, zu), 74, 94),
                    (layer_norm(Balanced, i + 2, F[u], zu), 0, 66)], 12, 8, 7)
                keys_values(i, u, pace)
                project(X[u], 0, to_f32(o_s, i), pace)
            return z
        lax.fori_loop(1 - rep, NB // 2 - 1, body, z0)

        @pl.when(rep == 0)
        def _():
            for p in (6, 7, 12, 13):
                w_copy(p).wait()
            start((), (14, 15))

        @pl.when(rep == 1)
        def _():
            for n in range(4 * NB):
                out_copy(n).wait()

        done, za, zb = [], z0 << NB, z0 << (NB + 1)
        ops = panel_ops(6, 0, za) + panel_ops(7, 1, za) + panel_ops(0, 6, zb) + panel_ops(1, 7, zb)
        a, b, c = (len(ops) * k // 100 for k in (45, 92, 98))
        keys_values(NB - 2, 0, Pacer(za, done, 4 * NP, [
            (ops[:a], 0, 100), (token_ops(Balanced, fb, 0, xb, za), 0, 92)], 6, 6, 2))
        keys_values(NB - 1, 1, Pacer(zb, done, 4 * NP, [
            (ops[a:b], 0, 100), (lin_accumulate(NB - 2, kf, za), 3, 50)], 6, 6, 2))
        project(xa, 0, to_f32(o_s, NB - 2), Pacer(za, done, 2 * NP, [
            (ops[b:c], 0, 100),
            (lin_accumulate(NB - 1 + zb, kf, zb) + lin_finalize() + lin_output(0, fa, za), 6, 95)], 8, 4, 2))
        project(xb, 0, to_f32(o_s, NB - 1), Pacer(zb, done, 2 * NP, [
            (ops[c:], 0, 100), (lin_output(1, fb, zb), 0, 95), (token_ops(Classic, fa, 0, xa, zb), 5, 92)], 8, 4, 2))

    def lin_out(z0):
        done = []
        for i in range(NB):
            u, z, norm = i % 2, z0 << i, i >= NB - 2
            project(X[u], 6, to_residual(i, False), Pacer(z, done, 2 * NP, [
                (token_ops(Classic, F[1 - u], 0, X[1 - u], z), 0, 90),
                (layer_norm(Classic, u, F[u], z) if norm else lin_output(i + 2, F[u], z), 0, 90)],
                9 if norm else 6, 6, 2))

    def mha_qkv(z0):
        def body(it, zc):
            done = []
            for u in range(2):
                i, z = 2 * it + u, zc << u
                pace = Pacer(z, done, 6 * NP, [
                    (token_ops(Classic, F[1 - u], 0, X[1 - u], z), 0, 86),
                    (layer_norm(Classic, jnp.minimum(i + 2, NB - 1), F[u], z), 0, 96),
                    ([t for r in range(4) for t in weight_ops(Classic, 2 + (i >> 2), (i & 3) * 4 + r, wc, i >> 2, z)],
                     0, 90)], 14, 8, 2)
                project(X[u], 12, to_transposed(vt_s, i), pace)
                project(X[u], 8, to_transposed(q_s, i), pace, QSCALE)
                project(X[u], 10, to_bf16(k_s, i), pace)
            return zc
        lax.fori_loop(0, NB // 2, body, z0)

    def q_rows(g, j, rows):
        return jnp.concatenate([q_s[g, j * (BQ // TM) + b, rows, :] for b in range(BQ // TM)], axis=1)

    def widen_q(g, head, j, token=None):
        q = q_rows(g, j, _at(head * (DH // 2), DH // 2))
        q = _bf(q if token is None else q | jnp.tile(token, (DH // 16, BQ // 128))).astype(F32)
        q = jnp.concatenate([q, q[:8]])
        for b in range(BQ // 128):
            (qa, qb)[j % 2][0, b] = q[:, b * 128:(b + 1) * 128]

    def spread_k(g, pair, u, z):
        def left(v, n):
            return jnp.concatenate([v[:, n:], v[:, :n]], axis=1)

        def skew(late):
            firsts = [(n * VP + 2) * CK - RG for n in range(NV)]
            k = jnp.concatenate([k_s[g, r // TM, pl.ds(r % TM // 2, RG // 2), :] for r in firsts])
            token = late()
            k = _bf(k if token is None else k | jnp.tile(token, (NV, 1))).astype(F32)
            row = lax.broadcasted_iota(jnp.int32, k.shape, 0)
            lane = lax.broadcasted_iota(jnp.int32, k.shape, 1) & (DH - 1)
            k = jnp.where(pair == 0, k, left(k, 2 * DH))
            for n in (1, 2, 4):
                k = jnp.where((row & n) == 0, k, jnp.where(lane < DH - n, left(k, n), left(k, 128 - DH + n)))
            kr_s[u] = pltpu.bitcast(k, U32)

        def task(d, late):
            k, token = kr_s[u + z * d], late()
            if token is not None:
                k = k | jnp.tile(token, (2 * NV, 1))
            (ka, kb)[u][0, d] = jnp.broadcast_to(k[:, u * DH + d:u * DH + d + 1], k.shape).reshape(-1, 8, 128)
        return [skew, lambda late: None] + [lambda late, d=d: task(d, late) for d in range(DH)]

    def stream(qk, c0, c1, pv, m, mx, z, extra, shared):
        steps, tiles = CK // RG, BQ // 128
        ms, mxu_scores, probs = [m], {}, {}
        st = dict(mx=mx, token=None, acc=None, l=None, stored=c0 * steps)
        zs, zero, nothing = _memo(lambda k: z * k), _zero_tile(z), jnp.zeros((8, 128), U32)
        head_rows = _memo(lambda t, h: _at(jnp.where(qk[t][1] == h // 2, h * (DH // 2), 64), DH // 2))

        def score_ref(j, row):
            return scores[j % 2 * NS + row // (S // NS)], row % (S // NS) // 8

        def score(ci):
            t, c = divmod(ci, NC)
            g, _, u, j = qk[t]
            keys = CK - RG if ci < shared and c % VP == 1 else CK
            k = k_s[g + zs(t + 1), c * CK // TM, pl.ds(c * CK % TM // 2, keys // 2), :]
            gq = g + zs(c + 1)
            q = {h: q_rows(gq, j, head_rows(t, h)) for h in (u, u + 2)}
            q = jnp.concatenate([q[h] if h in q else jnp.zeros_like(q[u]) for h in range(4)])
            mxu_scores[ci] = jnp.dot(_bf(k), _bf(q), preferred_element_type=F32)

        def vpu_term(ci, d):
            t, c = divmod(ci, NC)
            k = (ka, kb)[qk[t][2]][zs(t + 1), d, pl.ds(c // VP * 2, 2)]
            k = pltpu.bitcast(k if st["token"] is None else k | st["token"], F32)
            term = k[:, None] * (qa, qb)[qk[t][3] % 2][pl.ds(zs(c + 1), 1), :, pl.ds(d, 8), :]
            st["vpu"] = term if d == 0 else st["vpu"] + term

        def store_scores(upto):
            while st["stored"] < min(upto, c1 * steps):
                ci, k = divmod(st["stored"], steps)
                st["stored"] += 1
                t, c = divmod(ci, NC)
                if ci < shared:
                    ahead = (1 - ci) % VP
                    vpu_term(ci + ahead, (VP - 1 - ahead) * steps + k)
                for r in range(k * RG, (k + 1) * RG, 8):
                    if r < mxu_scores[ci].shape[0]:
                        s = mxu_scores[ci][r:r + 8]
                    else:
                        s = jnp.concatenate([st["vpu"][r % RG // 8, b] for b in range(tiles)], axis=1)
                    ref, row = score_ref(qk[t][3], c * CK + r)
                    ref[0, row] = s
                    st["mx"] = s if st["mx"] is None else jnp.maximum(st["mx"], s)
                    if r % RG == 0:
                        st["token"] = pltpu.bitcast(s[:, 256:384], U32) & zero
                if (c, k) == (NC - 1, steps - 1):
                    top = jnp.broadcast_to(jnp.max(st["mx"], axis=0, keepdims=True), (8, BQ))
                    ms.append(pltpu.bitcast(top, U32)[None])
                    st["mx"] = None

        def exponentiate(ci, token=None):
            t, c = divmod(ci, NC)
            parts = {}
            for k in reversed(range(steps)):
                store_scores((ci + c0) * steps - k - 1)
                if ci < c1 - c0:
                    token = st["token"]
                if token is not None:
                    every = ci >= c1 - c0 or (c, k) == (0, steps - 1)
                    ms[t] = ms[t] | jnp.concatenate(
                        [token if every or (b + k) % tiles == 0 else nothing for b in range(tiles)], axis=1)
                    token = None
                ref, row = score_ref(pv[t][3], c * CK + k * RG)
                parts[k] = jnp.exp2(ref[z, pl.ds(row, RG // 8)] - pltpu.bitcast(ms[t], F32))
                part = jnp.sum(parts[k], axis=0)
                st["l"] = part if st["l"] is None else st["l"] + part
            probs[ci] = jnp.concatenate([parts[k] for k in range(steps)]).reshape(CK, BQ).astype(BF)

        def weigh(ci):
            t, c = divmod(ci, NC)
            g, pair, u, j = pv[t]
            v = vt_s[g + zs(t + 1), c * CK // TM, _at(pair * DH + u * (DH // 2), DH // 2), pl.ds(c * CK % TM, CK)]
            o = jnp.dot(_bf(v), probs.pop(ci), preferred_element_type=F32)
            if c:
                o = acc_s[z] + o
            elif st["acc"] is not None:
                o = st["acc"] + o
            if c < NC - 1:
                acc_s[0] = o
            else:
                ot_s[u, j, :DH, :] = o
                ot_s[u, j, DH:, :] = st["l"]
                st["acc"] = pltpu.bitcast(pltpu.bitcast(o, jnp.int32) & z, F32)
                st["l"] = None

        for ci in range(c0, c1):
            if ci < shared and ci % NC == NC - 6:
                g, pair, u, j = qk[ci // NC + 1]
                widen_q(g, 2 * pair + u, j, st["token"])
            for tasks, first, end in extra:
                if first <= ci < end:
                    for task in _part(tasks, ci - first, end - first):
                        task(lambda: st["token"])
            score(ci)
            if pv:
                exponentiate(ci - c0)
                weigh(ci - c0)
        store_scores(c1 * steps)
        if st["mx"] is not None:
            m_s[0] = ms[-1][0]
            m_s[1] = pltpu.bitcast(st["mx"], U32)
        return [lambda late, n=n: (exponentiate(n, late()), weigh(n))[1] for n in range(c1 - c0, len(pv) * NC)]

    def normalize(slot, pair, u, j):
        def task(late):
            token = late()
            l = _after(ot_s[u, j, DH:, :], None if token is None else jnp.tile(token, (1, BQ // 128)))
            on_s[slot, j, _at((2 * pair + u) * DH, DH), :] = (
                ot_s[u, j, :DH, :] * (1.0 / jnp.sum(l, axis=0, keepdims=True)))
        return [task]

    def transpose_out(slot, g, j):
        def task(b, late):
            o = on_s[slot, j, :, pl.ds(b * 128, 128)]
            o = jnp.concatenate([_after(o[:8], late()), o[8:]])
            o_s[2 * j + b // 2, pl.ds(b % 2 * 2, 2), :, _at(g * 128, 128)] = o.T.reshape(2, MB, 128)
        return [lambda late, b=b: task(b, late) for b in range(BQ // 128)]

    def attention(z0):
        widen_q(0, 0, 1)
        stream([(0, 0, 0, 0), (0, 0, 0, 1)], 0, NC + 2, [], None, None, z0, [(spread_k(0, 0, 0, z0), 0, NC)], 0)

        def finish(j):
            return normalize(1, 1, 0, j) + normalize(1, 1, 1, j) + transpose_out(1, G - 1, j)

        def body(it, z, last=False):
            g, pair, m, mx = it >> 1, it & 1, m_s[:1], pltpu.bitcast(m_s[1], F32)
            items = [(g, pair, u, j) for u in range(2) for j in range(NQ)]
            prev = g - 1 if last else jnp.maximum(g - 1, 0)
            extra = [([t for u in range(2) for j in range(NQ)
                       for t in normalize(((it + 3) >> 1) & 1, 1 - pair, u, j)], 7, NC - 1),
                     (spread_k(g, pair, 1, z), 12, 3 * NC - 4),
                     (transpose_out(1 - (g & 1), prev, 2 * pair) + transpose_out(1 - (g & 1), prev, 2 * pair + 1),
                      *((3 * NC, 5 * NC) if last else (6 * NC + 8, 8 * NC - 6)))]
            if last:
                extra.append((finish(0), 5 * NC + 3, 5 * NC + 9))
                extra.append((token_ops(Classic, o_s, 0, xa, z), 5 * NC + 11, 7 * NC - 2))
                return stream(items[1:], 2, 7 * NC, items, m, mx, z, extra, 5 * NC + 2)
            g, pair = (it + 1) >> 1, (it + 1) & 1
            extra.append((spread_k(g, pair, 0, z), 3 * NC, 6 * NC + 8))
            stream(items[1:] + [(g, pair, 0, 0), (g, pair, 0, 1)], 2, 8 * NC + 2, items, m, mx, z, extra, 8 * NC + 2)
            return z
        lax.fori_loop(0, 2 * G - 1, body, z0)
        return finish(1) + body(2 * G - 1, z0, True) + finish(2) + finish(3)

    def mha_out(z0, pending):
        done = []
        for i in range(NB):
            u, z = i % 2, z0 << i
            ops = token_ops(Classic, o_s, i + 1, X[1 - u], z) if i < NB - 1 else token_ops(Balanced, fa, 0, xa, z)
            if i < 3:
                more, timing = _part(pending, i, 3), (6, 8, 2)
            else:
                more = (layer_norm(Balanced, 0, fa, z) + layer_norm(Balanced, 1, fb, z))[(i - 3) * 15:(i - 2) * 15]
                timing = (7, 6, 3)
            project(X[u], 14, to_residual(i, True), Pacer(z, done, 2 * NP, [(ops, 0, 90), (more, 0, 90)], *timing))

    def first_norm(i):
        def body(n, c):
            for r in range(0, TM // 2, 16):
                xc, rs = _centered(xs[i, _at(n * (TM // 2) + r, 16), :].astype(F32))
                xn_s[0, 2 * i + n, pl.ds(r // 2, 8), :] = _pack(xc * rs)
            return c
        lax.fori_loop(0, 2, body, 0)

    def first_panel(p, z, done, lists):
        tasks = [t for r in range(16) for t in weight_ops(Balanced, p, r, wa, p, z, False)]
        pace = Pacer(z, done, 64, [(tasks, 0, 99)] + lists, 2, 5, 2)
        for nj in range(4):
            for b in range(4):
                zx, slot, total = z * (nj + 1), p + z * (b + 8), None
                for k in range(4):
                    part = pace.dot(xn_s[zx, b, :, pl.ds(k * 256, 256)],
                                    raw[slot, pl.ds(2 * k, 2), :, pl.ds(nj * 128, 128)].reshape(256, 128))
                    total = part if total is None else total + part
                o_s[(p >> 1) * 2 + b // 2, pl.ds(b % 2 * 2, 2), :, _at((p & 1) * PW + nj * 128, 128)] = (
                    total.reshape(2, MB, 128))

    def first_v(i):
        def task(g, late):
            v = o_s[4 + i, :, :, pl.ds(g * 128, 128)].reshape(TM, 128)
            v = jnp.concatenate([_after(v[:8], late()), v[8:]])
            vt_s[g, i] = pltpu.bitcast(v.astype(BF).T, U32)
        return [lambda late, g=g: task(g, late) for g in range(G)]

    def kv_panel(p, c):
        w_wait(p)
        for n, nxt in enumerate((((), (3, 4)), ((), (5, 0)), ((2, 3), (1,)), ((4, 5), (8,)))):
            pl.when(p == 2 + n)(lambda nxt=nxt: start(*nxt))
        first_panel(p, p >> 3, [], [])
        return p >> 3

    start((0, 1), ())
    kv_s[...] = jnp.zeros(kv_s.shape, F32)
    z_s[...] = jnp.zeros(z_s.shape, F32)
    ot_s[...] = jnp.ones(ot_s.shape, F32)
    on_s[1, :, :64, :] = jnp.zeros((NQ, 64, BQ), F32)
    q_s[:, :, 64:, :] = jnp.zeros((G, NB, 16, TM), U32)
    x_copy(0).wait()
    start((), (2,))
    first_norm(0)
    x_copy(1).wait()
    first_norm(1)
    zero = lax.fori_loop(2, 6, kv_panel, 0)
    for copy in (x_copy(2), x_copy(3), w_copy(0), w_copy(1)):
        copy.wait()
    start((), (9, 10))
    finished = []
    for p in range(2):
        first_panel(p, zero << 4 * p, finished, [
            (layer_norm(Balanced, 2 + p, F[p], zero), 0, 50),
            (token_ops(Balanced, fa, 0, xa, zero), 0, 94) if p else (first_v(0) + first_v(1), 0, 50),
            (lin_accumulate(p, o_s, 2 + p), 50, 97)])
    start((6, 7), (11,))

    def layer_pair(rep, c):
        z0 = rep >> 1
        lin_qkv(rep, z0)
        lax.fori_loop(z0, 1, lambda z, _: lin_out(z), None)

        @pl.when(rep == 0)
        def _():
            w_copy(14).wait()
            w_copy(15).wait()

        mha_qkv(z0)
        mha_out(z0, attention(z0))
        return c
    lax.fori_loop(0, 2, layer_pair, 0)
    for n in range(4 * NB):
        out_copy(n).wait()


@jax.jit
def pallas_interleave_layers__linear_attn_block__mha_block__prompt_kernel(
    A_x: jax.Array,
    A_wqkv: jax.Array,
    A_wo: jax.Array,
    B_x: jax.Array,
    B_wqkv: jax.Array,
    B_wo: jax.Array,
):
    del B_x
    any_spec = pl.BlockSpec(memory_space=pl.ANY)
    out = pl.pallas_call(
        _kernel,
        out_shape=jax.ShapeDtypeStruct((NB, TM, D), BF),
        in_specs=[any_spec] * 5,
        out_specs=any_spec,
        scratch_shapes=[
            pltpu.VMEM((NB, TM, D), BF),
            pltpu.VMEM((12, G, 128, PW), BF),
            pltpu.VMEM((6, 7, 128, 7 * 128), U32),
            pltpu.VMEM((8, 7, 128, 7 * 128), U32),
            pltpu.VMEM((2, 7, 128, 7 * 128), U32),
            pltpu.VMEM((1, 7, 2, MB // 2, 7 * 128), U32),
            pltpu.VMEM((1, 7, 2, MB // 2, 7 * 128), U32),
            pltpu.VMEM((1, 4, MB, D), F32),
            pltpu.VMEM((1, 4, MB, D), F32),
            pltpu.VMEM((1, 4, MB, D), F32),
            pltpu.VMEM((1, 4, 64, D), U32),
            pltpu.VMEM((G, NB, 80, TM), U32),
            pltpu.VMEM((G, NB, TM // 2, 128), U32),
            pltpu.VMEM((G, NB, 64, TM), U32),
            pltpu.VMEM((NB, 4, MB, D), F32),
            pltpu.VMEM((G, 128, 128), F32),
            pltpu.VMEM((G, 8, 128), F32),
            pltpu.VMEM((G, 72, 128), U32),
            pltpu.VMEM((2, 8, BQ), U32),
            pltpu.VMEM((2, NQ, DH + 8, BQ), F32),
            pltpu.VMEM((2, NQ, 128, BQ), F32),
            pltpu.VMEM((1, DH, BQ), F32),
            pltpu.VMEM((2, RG * NV, 128), U32),
            pltpu.VMEM((1, DH, 2 * NV, 8, 128), U32),
            pltpu.VMEM((1, DH, 2 * NV, 8, 128), U32),
            pltpu.VMEM((1, BQ // 128, DH + 8, 128), F32),
            pltpu.VMEM((1, BQ // 128, DH + 8, 128), F32),
            pltpu.SemaphoreType.DMA((NB,)),
            pltpu.SemaphoreType.DMA((16,)),
            pltpu.SemaphoreType.DMA((4 * NB,)),
        ] + [pltpu.VMEM((1, S // NS // 8, 8, BQ), F32)] * (2 * NS),
        compiler_params=pltpu.CompilerParams(vmem_limit_bytes=122 * 2 ** 20),
    )(A_x.reshape(NB, TM, D), *[w.reshape(G, 128, -1) for w in (A_wqkv, A_wo, B_wqkv, B_wo)])
    return out.reshape(A_x.shape)
```
